```python
import jax
import jax.numpy as jnp

def _softmax(x, axis=-1):
    return jax.nn.softmax(x, axis=axis)
def _gelu(x):
    return jax.nn.gelu(x, approximate=True)
def _silu(x):
    return jax.nn.silu(x)
def _sigmoid(x):
    return jax.nn.sigmoid(x)
def _layernorm(x, axis=-1, eps=1e-5):
    m = jnp.mean(x, axis=axis, keepdims=True)
    v = jnp.var(x, axis=axis, keepdims=True)
    return (x - m) / jnp.sqrt(v + eps)
def _scatter_add(tgt, idx, src, axis=0):
    return tgt.at[idx].add(src)
def _segment_sum(src, seg, n):
    return jax.ops.segment_sum(src, seg, n)
class _Rng:
    def __init__(self, key):
        self._k = key
    def _next(self):
        self._k, sub = jax.random.split(self._k)
        return sub
    def normal(self, shape):
        return jax.random.normal(self._next(), shape, dtype=jnp.bfloat16)
    def randint(self, lo, hi, shape):
        return jax.random.randint(self._next(), shape, lo, hi, dtype=jnp.int32)
    def uniform(self, shape, lo=0.0, hi=1.0):
        return jax.random.uniform(self._next(), shape, jnp.bfloat16, lo, hi)
    def permutation(self, n):
        return jax.random.permutation(self._next(), n)


kernel_name = 'gated_mix__sliding_local_dilated__moe_arch_mod__prompt'

def setup_inputs():
    _rng = _Rng(jax.random.key(int.from_bytes(__import__("os").urandom(4), "little")))
    _w = (lambda a: (lambda t: t.astype(jnp.bfloat16) if jnp.issubdtype(t.dtype, jnp.floating) else t)(jnp.asarray(a)))
    def _A_setup():
        B, S, D = 1, 2048, 640
        return {
            "x": _w((lambda *s: _rng.normal(s) * 0.05)(B, S, D)),
            "wqkv": _w((lambda *s: _rng.normal(s) * 0.05)(D, 3 * D)),
            "wo": _w((lambda *s: _rng.normal(s) * 0.05)(D, D)),
        }
    _A_in = _A_setup()

    def _B_setup():
        B, S, D, F, C = 1, 2048, 640, 1728, 2
        return {
            "x": _w((lambda *s: _rng.normal(s) * 0.05)(B, S, D)),
            "w_r": _w((lambda *s: _rng.normal(s) * 0.05)(D)),
            "w_gate": _w((lambda *s: _rng.normal(s) * 0.05)(D, F)),
            "w_up": _w((lambda *s: _rng.normal(s) * 0.05)(D, F)),
            "w_down": _w((lambda *s: _rng.normal(s) * 0.05)(F, D)),
        }
    _B_in = _B_setup()

    return {
        "A_x": _A_in["x"],
        "A_wqkv": _A_in["wqkv"],
        "A_wo": _A_in["wo"],
        "B_x": _B_in["x"],
        "B_w_r": _B_in["w_r"],
        "B_w_gate": _B_in["w_gate"],
        "B_w_up": _B_in["w_up"],
        "B_w_down": _B_in["w_down"],
        "gate_w": _w((lambda *s: _rng.normal(s) * 0.05)(640)),
    }

def reference(A_x, A_wqkv, A_wo, B_x, B_w_r, B_w_gate, B_w_up, B_w_down, gate_w):
    def _A_ref(x, wqkv, wo):
        B, S, D = x.shape
        H = 32; Dh = D // H
        W, dil = 8, 2
        qkv = (lambda x, *d: x.transpose(*d))((x @ wqkv).reshape(B, S, 3, H, Dh), 2, 0, 3, 1, 4)
        q, k, v = qkv[0], qkv[1], qkv[2]
        scale = Dh ** -0.5
        pos = jnp.arange(S)
        off = jnp.arange(W) * dil
        idx = pos[:, None] - off[None, :]
        mask = idx >= 0
        idx_c = jnp.where(mask, idx, 0).reshape(-1)
        kg = k[:, :, idx_c, :].reshape(B, H, S, W, Dh)
        vg = v[:, :, idx_c, :].reshape(B, H, S, W, Dh)
        logits = jnp.einsum("bhsd,bhswd->bhsw", q, kg) * scale
        logits = jnp.where(mask[None, None, :, :], logits, -1e9)
        attn = _softmax(logits, axis=-1)
        o = jnp.einsum("bhsw,bhswd->bhsd", attn, vg)
        return (lambda x, *d: x.transpose(*d))(o, 0, 2, 1, 3).reshape(B, S, D) @ wo

    def _B_ref(x, w_r, w_gate, w_up, w_down):
        B, S, D = x.shape
        C = 2
        r = x @ w_r
        idx = jnp.argsort(-r, axis=-1)[:, :C]
        idx_e = jnp.repeat(idx.reshape(B, C, 1), D, axis=2)
        x_sel = jnp.take_along_axis(x, idx_e, axis=1)
        g = _silu(x_sel @ w_gate)
        u = x_sel @ w_up
        y = (g * u) @ w_down
        r_sel = _sigmoid(jnp.take_along_axis(r, idx, axis=1))
        y = y * r_sel.reshape(B, C, 1)
        b_off = (jnp.arange(B) * S).reshape(B, 1)
        flat_idx = (idx + b_off).reshape(B * C)
        zero = (x * 0.0).reshape(B * S, D)
        upd = _scatter_add(zero, flat_idx, y.reshape(B * C, D), axis=0)
        return x + upd.reshape(B, S, D)

    x = A_x
    g = _sigmoid((x * gate_w).sum(-1, keepdims=True))
    a = _A_ref(x, A_wqkv, A_wo)
    b = _B_ref(x, B_w_r, B_w_gate, B_w_up, B_w_down)
    return g * a + (1 - g) * b
```

```python
import jax
import jax.numpy as jnp
from jax import lax
import jax.experimental.pallas as pl
import jax.experimental.pallas.tpu as pltpu

S, D, F = 2048, 640, 1728
H, DH, W = 32, 20, 8
NT = D // 128
T = 256
NC = S // T
NI = T // 16
HALO = (W - 1) * 16
SCALE = DH ** -0.5
LOG2E = 1.4426950408889634
KB = ((0, 256), (256, 256), (512, 128))

f32, bf16, u32, i32 = jnp.float32, jnp.bfloat16, jnp.uint32, jnp.int32


def _sigmoid(x):
    return 1.0 / (1.0 + jnp.exp(-x))


def _lane_masks(rows):
    lane = lax.broadcasted_iota(i32, (rows, 128), 1)
    lo = lane < 64
    even = (lane & 32) == 0
    mid = (lane >= 32) & (lane < 96)
    return lane, lo, even, mid


def _fold4(p, masks):
    _, lo, even, mid = masks
    c = jnp.where(lo, p[0], p[1]) + pltpu.roll(jnp.where(lo, p[1], p[0]), 64, 1)
    d = jnp.where(mid, p[2], p[3]) + pltpu.roll(jnp.where(mid, p[3], p[2]), 64, 1)
    return jnp.where(even, c, d) + pltpu.roll(jnp.where(even, d, c), 96, 1)


def _spread4(e, masks):
    _, lo, even, mid = masks
    f = pltpu.roll(e, 32, 1)
    c = jnp.where(even, e, f)
    d = jnp.where(even, f, e)
    cr = pltpu.roll(c, 64, 1)
    dr = pltpu.roll(d, 64, 1)
    return [jnp.where(lo, c, cr), jnp.where(lo, cr, c),
            jnp.where(mid, d, dr), jnp.where(mid, dr, d)]


def _kernel(ax_hbm, wqkv_hbm, wo_hbm, wr_ref, wg_hbm, wu_hbm, wd_hbm, gw_ref,
            out_hbm,
            xa, gate, wraw, wp, woraw, wop, wg, wu, wd, tmp, tmpf,
            qs, ks, vs, ob, outb, rkeys, sems):
    xa32 = xa.bitcast(u32)
    ob32 = ob.bitcast(u32)

    n_sem = [0]

    def copy(src, dst):
        c = pltpu.make_async_copy(src, dst, sems.at[n_sem[0]])
        n_sem[0] += 1
        return c

    def x_copies(r0, n):
        return [copy(ax_hbm.at[pl.ds(r0, n), pl.ds(128 * j, 128)], xa.at[j, pl.ds(r0, n), :])
                for j in range(NT)]

    cp_w = [[copy(wqkv_hbm.at[pl.ds(r0, n), pl.ds(D * p, D)], wraw.at[pl.ds(r0, n), pl.ds(D * p, D)])
             for (r0, n) in KB] for p in range(3)]
    x_pieces = ((0, T), (T, T), (2 * T, 2 * T), (4 * T, 4 * T))
    cp_x = [x_copies(r0, n) for (r0, n) in x_pieces]
    cp_wo = copy(wo_hbm, woraw)
    cp_wg = copy(wg_hbm, wg)
    cp_wu = copy(wu_hbm, wu)
    cp_wd = copy(wd_hbm, wd)
    cp_out = [copy(outb.at[pl.ds(c * T, T), :], out_hbm.at[pl.ds(c * T, T), :]) for c in range(NC)]

    def start(cs):
        for c in cs:
            c.start()

    def wait(cs):
        for c in cs:
            c.wait()

    def permute_wqkv(p, b):
        r0, n = KB[b]
        w = pltpu.bitcast(wraw[pl.ds(r0, n), pl.ds(D * p, D)], u32)
        if n == 128:
            w = jnp.concatenate([w, jnp.zeros_like(w)], axis=0)
        slot = 3 * p + b
        tmp[slot] = w.T
        perm = jnp.concatenate(
            [tmp[slot, pl.ds(d, H, stride=DH), :] for d in range(DH)], axis=0)
        wp[pl.ds(r0, n), pl.ds(D * p, D)] = pltpu.bitcast(perm.T[: n // 2], bf16)

    def permute_wo(j):
        tmpf[j] = woraw[:, pl.ds(128 * j, 128)].astype(f32)
        perm = jnp.concatenate(
            [tmpf[j, pl.ds(d, H, stride=DH), :] for d in range(DH)], axis=0)
        wop[:, pl.ds(128 * j, 128)] = perm.astype(bf16)

    def load_x(c):
        cols = []
        for j in range(NT):
            rows = [xa32[j, pl.ds(c * (T // 2) + i, 8, stride=NI), :] for i in range(NI)]
            cols.append(pltpu.bitcast(jnp.concatenate(rows, axis=0), bf16))
        return jnp.concatenate(cols, axis=1)

    def project(c, p):
        y = jnp.dot(load_x(c), wp[:, pl.ds(D * p, D)], preferred_element_type=f32)
        if p == 0:
            qs[c] = y
            return
        dst = ks if p == 1 else vs
        dst[c, pl.ds(HALO, T), :] = y
        row = lax.broadcasted_iota(i32, (8, D), 0)
        for i in range(NI - (W - 1), NI):
            lo8 = pltpu.roll(y[16 * i: 16 * i + 8], 2, 0)
            hi8 = pltpu.roll(y[16 * i + 8: 16 * i + 16], 2, 0)
            if c > 0:
                prev = pltpu.roll(dst[c - 1, pl.ds(HALO + 16 * i + 8, 8), :], 2, 0)
            else:
                prev = jnp.broadcast_to(y[0:1], (8, D))
            h0 = 16 * (i - (NI - (W - 1)))
            dst[c, pl.ds(h0, 8), :] = jnp.where(row < 2, prev, lo8)
            dst[c, pl.ds(h0 + 8, 8), :] = jnp.where(row < 2, lo8, hi8)

    def attend(c, i):
        masks = _lane_masks(16)
        lane = masks[0]
        r0 = 16 * i
        q = [qs[c, pl.ds(r0, 16), pl.ds(128 * j, 128)] for j in range(NT)]
        part = []
        for w in range(W):
            acc = None
            for j in range(NT):
                t = q[j] * ks[c, pl.ds(HALO + r0 - 16 * w, 16), pl.ds(128 * j, 128)]
                acc = t if acc is None else acc + t
            part.append(acc)
        ea = _fold4(part[:4], masks)
        eb = _fold4(part[4:], masks)
        masked = c == 0 and i < W - 1
        if masked:
            grp = lane >> 5
            w_lane = ((grp & 1) << 1) | (grp >> 1)
            first = lax.broadcasted_iota(i32, (16, 128), 0) < 2
            ea = jnp.where(first & (w_lane > i), -1e9, ea * SCALE)
            eb = jnp.where(first & (w_lane + 4 > i), -1e9, eb * SCALE)
        m = jnp.maximum(ea, eb)
        m = jnp.maximum(m, pltpu.roll(m, 64, 1))
        m = jnp.maximum(m, pltpu.roll(m, 32, 1))
        cst = LOG2E if masked else SCALE * LOG2E
        ea = jnp.exp2((ea - m) * cst)
        eb = jnp.exp2((eb - m) * cst)
        s = ea + eb
        s = s + pltpu.roll(s, 64, 1)
        s = s + pltpu.roll(s, 32, 1)
        inv = 1.0 / s
        prob = _spread4(ea * inv, masks) + _spread4(eb * inv, masks)
        for j in range(NT):
            acc = None
            for w in range(W):
                t = prob[w] * vs[c, pl.ds(HALO + r0 - 16 * w, 16), pl.ds(128 * j, 128)]
                acc = t if acc is None else acc + t
            ob32[j, pl.ds(c * (T // 2) + i, 8, stride=NI), :] = pltpu.bitcast(acc.astype(bf16), u32)

    def router(c):
        rows = pl.ds(c * T, T)
        wr = wr_ref[...].reshape(1, D).astype(f32)
        gw = gw_ref[...].reshape(1, D).astype(f32)
        acc = gacc = None
        for j in range(NT):
            x = xa[j, rows, :].astype(f32)
            t = x * wr[:, 128 * j: 128 * (j + 1)]
            u = x * gw[:, 128 * j: 128 * (j + 1)]
            acc = t if acc is None else acc + t
            gacc = u if gacc is None else gacc + u
        g = _sigmoid(jnp.sum(gacc, axis=1, keepdims=True))
        gate[rows, :] = jnp.broadcast_to(g, (T, 128))
        r = jnp.sum(acc.T, axis=0, keepdims=True)
        r = r.astype(bf16).astype(f32) + 0.0
        bits = pltpu.bitcast(r, i32)
        bits = jnp.where(bits < 0, bits ^ 0x7FFF0000, bits)
        pos = c * T + lax.broadcasted_iota(i32, (1, T), 1)
        rkeys[pl.ds(c, 1), :] = bits | (0xFFFF - pos)

    def select():
        keys = rkeys[...]
        k0 = jnp.max(keys)
        k1 = jnp.max(jnp.where(keys == k0, jnp.iinfo(jnp.int32).min, keys))
        return k0, k1

    def row_tile(key):
        idx = 0xFFFF - (key & 0xFFFF)
        idx = jnp.clip(idx, 0, S - 1)
        base = pl.multiple_of((idx >> 4) << 4, 16)
        return base, idx & 15

    def x_tile(base):
        return jnp.concatenate(
            [xa[j, pl.ds(base, 16), :] for j in range(NT)], axis=1).astype(f32)

    def gather(sel):
        row = lax.broadcasted_iota(i32, (16, D), 0)
        x_sel = jnp.zeros((16, D), f32)
        for n, key in enumerate(sel):
            base, sub = row_tile(key)
            tile = x_tile(base)
            picked = jnp.sum(jnp.where(row == sub, tile, 0.0), axis=0, keepdims=True)
            x_sel = jnp.where(row == n, picked, x_sel)
        return x_sel.astype(bf16)

    def ffn_up(x_sel):
        nt = (((1,), (1,)), ((), ()))
        g = lax.dot_general(x_sel, wg[...], nt, preferred_element_type=f32)
        u = lax.dot_general(x_sel, wu[...], nt, preferred_element_type=f32)
        return (g * _sigmoid(g) * u).astype(bf16)

    def ffn_down(h, sel):
        y = jnp.dot(h, wd[...], preferred_element_type=f32)
        row = lax.broadcasted_iota(i32, (16, D), 0)
        for n, key in enumerate(sel):
            base, sub = row_tile(key)
            kv = jnp.full((1, D), key, i32) & -65536
            r = pltpu.bitcast(jnp.where(kv < 0, kv ^ 0x7FFF0000, kv), f32)
            upd = y[n: n + 1] * _sigmoid(r)
            tile = x_tile(base)
            tile = jnp.where(row == sub, tile + upd, tile).astype(bf16)
            for j in range(NT):
                xa[j, pl.ds(base, 16), :] = tile[:, 128 * j: 128 * (j + 1)]

    def finish(c):
        rows = pl.ds(c * T, T)
        o = jnp.concatenate([ob[j, rows, :] for j in range(NT)], axis=1)
        a = jnp.dot(o, wop[...], preferred_element_type=f32)
        g = gate[rows, :]
        for j in range(NT):
            cols = slice(128 * j, 128 * (j + 1))
            b = xa[j, rows, :].astype(f32)
            outb[rows, cols] = (g * a[:, cols] + (1.0 - g) * b).astype(bf16)
        cp_out[c].start()

    def attend_chunk(c):
        for i in range(NI):
            attend(c, i)

    start(cp_w[0])
    start(cp_x[0])
    start(cp_w[1])
    start(cp_w[2])
    start(cp_x[1])
    start(cp_x[2])
    start(cp_x[3])
    start([cp_wo, cp_wg, cp_wu, cp_wd])

    for p in range(3):
        for b in range(3):
            cp_w[p][b].wait()
            permute_wqkv(p, b)
        if p == 0:
            wait(cp_x[0])
        project(0, p)

    sel = h = None
    for t in range(1, NC):
        if t in (1, 2, 3):
            wait(cp_x[t])
        if t == 5:
            cp_wo.wait()
        if t == 6:
            wait([cp_wg, cp_wu])
        if t == 7:
            cp_wd.wait()
        for p in range(3):
            project(t, p)
        attend_chunk(t - 1)
        if t <= 4:
            router(2 * t - 2)
            router(2 * t - 1)
        if t == 5:
            sel = select()
            for j in range(NT):
                permute_wo(j)
        if t == 6:
            h = ffn_up(gather(sel))
        if t == 7:
            ffn_down(h, sel)
    attend_chunk(NC - 1)
    for c in range(NC):
        finish(c)
    wait(cp_out)


@jax.jit
def pallas_gated_mix__sliding_local_dilated__moe_arch_mod__prompt_kernel(
    A_x: jax.Array,
    A_wqkv: jax.Array,
    A_wo: jax.Array,
    B_x: jax.Array,
    B_w_r: jax.Array,
    B_w_gate: jax.Array,
    B_w_up: jax.Array,
    B_w_down: jax.Array,
    gate_w: jax.Array,
):
    del B_x
    hbm = pl.BlockSpec(memory_space=pltpu.HBM)
    vmem = pl.BlockSpec(memory_space=pltpu.VMEM)
    out = pl.pallas_call(
        _kernel,
        in_specs=[hbm, hbm, hbm, vmem, hbm, hbm, hbm, vmem],
        out_specs=hbm,
        out_shape=jax.ShapeDtypeStruct((S, D), bf16),
        scratch_shapes=[
            pltpu.VMEM((NT, S, 128), bf16),
            pltpu.VMEM((S, 128), f32),
            pltpu.VMEM((D, 3 * D), bf16),
            pltpu.VMEM((D, 3 * D), bf16),
            pltpu.VMEM((D, D), bf16),
            pltpu.VMEM((D, D), bf16),
            pltpu.VMEM((F, D), bf16),
            pltpu.VMEM((F, D), bf16),
            pltpu.VMEM((F, D), bf16),
            pltpu.VMEM((9, D, 128), u32),
            pltpu.VMEM((NT, D, 128), f32),
            pltpu.VMEM((NC, T, D), f32),
            pltpu.VMEM((NC, HALO + T, D), f32),
            pltpu.VMEM((NC, HALO + T, D), f32),
            pltpu.VMEM((NT, S, 128), bf16),
            pltpu.VMEM((S, D), bf16),
            pltpu.VMEM((NC, T), i32),
            pltpu.SemaphoreType.DMA((48,)),
        ],
        compiler_params=pltpu.CompilerParams(vmem_limit_bytes=100 * 1024 * 1024),
    )(A_x.reshape(S, D), A_wqkv, A_wo, B_w_r, B_w_gate.T, B_w_up.T, B_w_down, gate_w)
    return out.reshape(1, S, D)
```

```python
import jax
import jax.numpy as jnp
from jax import lax
import jax.experimental.pallas as pl
import jax.experimental.pallas.tpu as pltpu

S, D, F = 2048, 640, 1728
H, DH, W = 32, 20, 8
NT = D // 128
T = 256
NC = S // T
NI = T // 16
HALO = (W - 1) * 16
SCALE = DH ** -0.5
LOG2E = 1.4426950408889634
KB = ((0, 256), (256, 256), (512, 128))

AN, SN, VN = 16, 128, 16
FP = 128
ROUTE, WO_AT = 6, 5
OUT_BLOCKS = [(r0, T) for r0 in range(0, S, T)]
R, B = 8, 3500
FENCE = 100
TICK, RT = 3.2, 1
HEAD = [(("wq",), 0, 0), (("x0_wk",), 0, 200), ((), 5, 0), (("wv",), 5, 0), (("x1",), 6, B)]
ARRIVALS = [(32, "x2_wo"), (56, "ffn")]

f32, bf16, u32, i32 = jnp.float32, jnp.bfloat16, jnp.uint32, jnp.int32


def _sigmoid(x):
    return 0.5 * jnp.tanh(0.5 * x) + 0.5


def _packed(x):
    return pltpu.bitcast(x, u32)


def _unpacked(x):
    return pltpu.bitcast(x, bf16)


def _lane_masks(rows):
    lane = lax.broadcasted_iota(i32, (rows, 128), 1)
    lo = lane < 64
    even = (lane & 32) == 0
    mid = (lane >= 32) & (lane < 96)
    return lane, lo, even, mid


def _fold4(p, masks):
    _, lo, even, mid = masks
    c = jnp.where(lo, p[0], p[1]) + pltpu.roll(jnp.where(lo, p[1], p[0]), 64, 1)
    d = jnp.where(mid, p[2], p[3]) + pltpu.roll(jnp.where(mid, p[3], p[2]), 64, 1)
    return jnp.where(even, c, d) + pltpu.roll(jnp.where(even, d, c), 96, 1)


def _spread4(e, masks):
    _, lo, even, mid = masks
    f = pltpu.roll(e, 32, 1)
    c = jnp.where(even, e, f)
    d = jnp.where(even, f, e)
    cr = pltpu.roll(c, 64, 1)
    dr = pltpu.roll(d, 64, 1)
    return [jnp.where(lo, c, cr), jnp.where(lo, cr, c),
            jnp.where(mid, d, dr), jnp.where(mid, dr, d)]


def _interleave(*lists):
    order = sorted(((k + 0.5) / len(l), n, k) for n, l in enumerate(lists) for k in range(len(l)))
    return [lists[n][k] for _, n, k in order]


def _schedule():
    matrix = [(("project", c, n), [("permute_x", c, j) for j in range(NT)]
               + [("permute_wqkv", n // NT, b) for b in range(len(KB))])
              for c in range(NC) for n in range(3 * NT)]
    for r0, n in OUT_BLOCKS:
        deps = ([("mix_values", r // T, r % T, VN) for r in range(r0 // T * T, r0 // T * T + T, VN)]
                + [("scatter",)] + [("permute_wo", j) for j in range(NT)])
        matrix += [(("finish", r0, n, j), deps) for j in range(NT)]

    vector = []
    for p, data in enumerate(("wq", "x0_wk", "wv")):
        vector += [(("permute_wqkv", p, b), 0, [data]) for b in range(len(KB))]
    x_data = ["x0_wk"] + ["x1"] * 3 + ["x2_wo"] * 4
    for c in range(NC):
        deps = [x_data[c]] + ([("project", c - 2, 3 * NT - 1)] if c > 1 else [])
        vector += [(("permute_x", c, j), 30, deps) for j in range(NT)]
    units = [(f0, min(FP, F - f0)) for f0 in range(0, F, FP)]
    routers = [("router", r0) for r0 in range(0, S, 128)]
    vector += [(("select",), 300, routers)]
    ups = [("ffn_up", *u, which) for u in units for which in range(2)]
    vector += [(t, None, [("select",), "ffn"]) for t in ups]
    vector += [(("ffn_down", *u), None, [("ffn_up", *u, 1)]) for u in units]
    vector += [(("scatter",), 100, [("ffn_down", *u) for u in units]
                + [("permute_x", NC - 1, j) for j in range(NT)])]
    for c in range(NC):
        ready = [("project", c, n) for n in range(2 * NT)]
        vector += [(("scores", c, r, AN), 72 * AN // 8, ready) for r in range(0, T, AN)]
        vector += [(("softmax", c, r, SN), 55 * SN // 8,
                    [("scores", c, a, AN) for a in range(r // AN * AN, r + SN, AN)])
                   for r in range(0, T, SN)]
        vector += [(("mix_values", c, r, VN), 78 * VN // 8,
                    [("softmax", c, r // SN * SN, SN), ("project", c, 3 * NT - 1)])
                   for r in range(0, T, VN)]
        for t in routers[c * ROUTE: (c + 1) * ROUTE]:
            vector += [(t, 500, ["x1", x_data[t[1] // T]])]
        if c == WO_AT:
            vector += [(("permute_wo", j), 150, ["x2_wo"]) for j in range(NT)]

    plan, done = [], []
    head, arrivals, issued = list(HEAD), list(ARRIVALS), 0
    while matrix or vector:
        if head:
            waits, pieces, budget = head.pop(0)
        else:
            waits, pieces, budget = (), R, B
            if arrivals and issued >= arrivals[0][0]:
                waits = (arrivals.pop(0)[1],)
        done += list(waits)
        if not vector:
            pieces = len(matrix)
        now = []
        for task, deps in matrix[:pieces]:
            if not all(d in done for d in deps):
                break
            now.append(task)
        picked, small, left = [], [], []
        for item in vector:
            task, cost, deps = item
            ready = all(d in done for d in deps)
            if ready and cost is None and len(small) < max(len(now), 1):
                small.append(task)
            elif ready and cost is not None and cost <= budget:
                picked.append(task)
                budget -= cost
            else:
                left.append(item)
        plan.append((waits, _interleave(now, small, picked)))
        done += now + small + picked
        issued += len(now)
        matrix, vector = matrix[len(now):], left
    return plan


def _kernel(ax_hbm, wqkv_hbm, wo_hbm, wr_hbm, wg_hbm, wu_hbm, wd_hbm, gw_hbm,
            out_hbm,
            xa, wraw, woraw, wg, wu, wd, wr_ref, gw_ref, rkeys, tmp, tmpf,
            wp, xp, qkv, logits, probs, ob, gate, outb, zeros, fence, sems):
    xa32 = xa.bitcast(u32)
    wraw32, woraw32, wg32, wu32, wd32 = (r.bitcast(u32) for r in (wraw, woraw, wg, wu, wd))

    def rows_bf16(ref32, j, r0, n):
        return _unpacked(ref32[j, pl.ds(r0 // 2, n // 2), :])

    def wide_bf16(ref32, j0, r0, n):
        return jnp.concatenate([rows_bf16(ref32, j0 + j, r0, n) for j in range(NT)], axis=1)

    n_sem = [0]

    def copy(src, dst):
        c = pltpu.make_async_copy(src, dst, sems.at[n_sem[0]])
        n_sem[0] += 1
        return c

    def tiles_in(src, dst, rows, tiles):
        return [copy(src.at[rows, pl.ds(128 * j, 128)], dst.at[j, rows, :]) for j in tiles]

    cp_w = [tiles_in(wqkv_hbm, wraw, pl.ds(0, D), range(NT * p, NT * p + NT)) for p in range(3)]
    x_pieces = ((0, T), (T, 3 * T), (4 * T, 4 * T))
    cp_x = [[copy(ax_hbm.at[pl.ds(r0, n), pl.ds(128 * j, 128)], xa.at[j, pl.ds(r0, n), :])
             for j in range(NT)] for (r0, n) in x_pieces]
    cp_wo = tiles_in(wo_hbm, woraw, pl.ds(0, D), range(NT))
    cp_wg = tiles_in(wg_hbm, wg, pl.ds(0, F), range(NT))
    cp_wu = tiles_in(wu_hbm, wu, pl.ds(0, F), range(NT))
    cp_wd = tiles_in(wd_hbm, wd, pl.ds(0, F), range(NT))
    cp_vec = [copy(wr_hbm, wr_ref), copy(gw_hbm, gw_ref)]
    cp_out = []

    def start(cs):
        for c in cs:
            c.start()

    def wait(cs):
        for c in cs:
            c.wait()

    def permute_wqkv(p, b):
        r0, n = KB[b]
        slot = 3 * p + b
        for j in range(NT):
            w = wraw32[NT * p + j, pl.ds(r0 // 2, n // 2), :]
            if n == 128:
                w = jnp.concatenate([w, jnp.zeros_like(w)], axis=0)
            tmp[slot][pl.ds(128 * j, 128), :] = w.T
        for j in range(NT):
            perm = jnp.concatenate(
                [tmp[slot][pl.ds(d, H, stride=DH), :] for d in range(4 * j, 4 * j + 4)], axis=0)
            wp[NT * p + j][pl.ds(r0 // 2, n // 2), :] = perm.T[: n // 2]

    def permute_wo(j):
        tmpf[j][...] = rows_bf16(woraw32, j, 0, D).astype(f32)
        perm = jnp.concatenate(
            [tmpf[j][pl.ds(d, H, stride=DH), :] for d in range(DH)], axis=0)
        wp[3 * NT + j][...] = _packed(perm.astype(bf16))

    def permute_x(c, j):
        rows = [xa32[j, pl.ds(c * (T // 2) + i, 8, stride=NI), :] for i in range(NI)]
        xp[c][j] = jnp.concatenate(rows, axis=0)

    def project(c, n):
        y = jnp.dot(wide_bf16(xp[c], 0, 0, T), _unpacked(wp[n][...]), preferred_element_type=f32)
        p, j = divmod(n, NT)
        dst = qkv[c][p]
        if p == 0:
            dst[j] = y
            return
        dst[j, pl.ds(HALO, T), :] = y
        row = lax.broadcasted_iota(i32, (8, 128), 0)
        for i in range(NI - (W - 1), NI):
            lo8 = pltpu.roll(y[16 * i: 16 * i + 8], 2, 0)
            hi8 = pltpu.roll(y[16 * i + 8: 16 * i + 16], 2, 0)
            if c > 0:
                prev = pltpu.roll(qkv[c - 1][p][j, pl.ds(HALO + 16 * i + 8, 8), :], 2, 0)
            else:
                prev = jnp.broadcast_to(y[0:1], (8, 128))
            h0 = 16 * (i - (NI - (W - 1)))
            dst[j, pl.ds(h0, 8), :] = jnp.where(row < 2, prev, lo8)
            dst[j, pl.ds(h0 + 8, 8), :] = jnp.where(row < 2, lo8, hi8)

    def scores(c, r0, n):
        q = [qkv[c][0][j, pl.ds(r0, n), :] for j in range(NT)]
        for w in range(W):
            acc = None
            for j in range(NT):
                t = q[j] * qkv[c][1][j, pl.ds(HALO + r0 - 16 * w, n), :]
                acc = t if acc is None else acc + t
            logits[c][w, pl.ds(r0, n), :] = acc
        return acc

    def softmax(c, r0, n):
        masks = _lane_masks(n)
        part = [logits[c][w, pl.ds(r0, n), :] for w in range(W)]
        ea, eb = _fold4(part[:4], masks), _fold4(part[4:], masks)
        masked = c == 0 and r0 < HALO
        if masked:
            grp = lax.broadcasted_iota(i32, (n, 128), 1) >> 5
            w_lane = ((grp & 1) << 1) | (grp >> 1)
            row = r0 + lax.broadcasted_iota(i32, (n, 128), 0)
            first = (row & 15) < 2
            ea = jnp.where(first & (w_lane > (row >> 4)), -1e9, ea * SCALE)
            eb = jnp.where(first & (w_lane + 4 > (row >> 4)), -1e9, eb * SCALE)
        m = jnp.maximum(ea, eb)
        m = jnp.maximum(m, pltpu.roll(m, 64, 1))
        m = jnp.maximum(m, pltpu.roll(m, 32, 1))
        cst = LOG2E if masked else SCALE * LOG2E
        ea = jnp.exp2((ea - m) * cst)
        eb = jnp.exp2((eb - m) * cst)
        s = ea + eb
        s = s + pltpu.roll(s, 64, 1)
        s = s + pltpu.roll(s, 32, 1)
        inv = pl.reciprocal(s, approx=True)
        inv = inv * (2.0 - s * inv)
        for w, v in enumerate(_spread4(ea * inv, masks) + _spread4(eb * inv, masks)):
            probs[c][w, pl.ds(r0, n), :] = v

    def mix_values(c, r0, n):
        prob = [probs[c][w, pl.ds(r0, n), :] for w in range(W)]
        for j in range(NT):
            acc = None
            for w in range(W):
                t = prob[w] * qkv[c][2][j, pl.ds(HALO + r0 - 16 * w, n), :]
                acc = t if acc is None else acc + t
            o = _packed(acc.astype(bf16))
            for k in range(n // 16):
                ob[c][j, pl.ds(r0 // 16 + k, 8, stride=NI), :] = o[8 * k: 8 * k + 8]
        return o

    def router(r0):
        wr = wr_ref[...].reshape(1, D).astype(f32)
        gw = gw_ref[...].reshape(1, D).astype(f32)
        acc = gacc = None
        for j in range(NT):
            x = rows_bf16(xa32, j, r0, 128).astype(f32)
            t = x * wr[:, 128 * j: 128 * (j + 1)]
            u = x * gw[:, 128 * j: 128 * (j + 1)]
            acc = t if acc is None else acc + t
            gacc = u if gacc is None else gacc + u
        g = _sigmoid(jnp.sum(gacc, axis=1, keepdims=True))
        gate[r0 // T][pl.ds(r0 % T, 128), :] = jnp.broadcast_to(g, (128, 128))
        r = jnp.sum(acc.T, axis=0, keepdims=True)
        r = r.astype(bf16).astype(f32) + 0.0
        bits = pltpu.bitcast(r, i32)
        bits = jnp.where(bits < 0, bits ^ 0x7FFF0000, bits)
        pos = r0 + lax.broadcasted_iota(i32, (1, 128), 1)
        rkeys[pl.ds(r0 // 128, 1), :] = bits | (0xFFFF - pos)

    state = {}

    def select():
        keys = rkeys[...]
        k0 = jnp.max(keys)
        k1 = jnp.max(jnp.where(keys == k0, jnp.iinfo(jnp.int32).min, keys))
        state["sel"] = (k0, k1)

    def row_tile(key):
        idx = jnp.clip(0xFFFF - (key & 0xFFFF), 0, S - 1)
        return pl.multiple_of((idx >> 4) << 3, 8), idx & 15

    def x_tile(base):
        return jnp.concatenate(
            [_unpacked(xa32[j, pl.ds(base, 8), :]) for j in range(NT)], axis=1).astype(f32)

    def gather():
        row = lax.broadcasted_iota(i32, (16, D), 0)
        x_sel = jnp.zeros((16, D), f32)
        for n, key in enumerate(state["sel"]):
            base, sub = row_tile(key)
            picked = jnp.sum(jnp.where(row == sub, x_tile(base), 0.0), axis=0, keepdims=True)
            x_sel = jnp.where(row == n, picked, x_sel)
        state["x_sel"] = x_sel.astype(bf16)

    def ffn_up(f0, n, which):
        w_t = wide_bf16(wu32 if which else wg32, 0, f0, n)
        y = lax.dot_general(state["x_sel"], w_t, (((1,), (1,)), ((), ())),
                            preferred_element_type=f32)
        if which == 0:
            state["g", f0] = y * _sigmoid(y)
        else:
            state["h", f0] = (state["g", f0] * y).astype(bf16)

    def ffn_down(f0, n):
        w = wide_bf16(wd32, 0, f0, n)
        y = jnp.dot(state["h", f0], w, preferred_element_type=f32)
        state["y"] = y if f0 == 0 else state["y"] + y

    def scatter():
        row = lax.broadcasted_iota(i32, (16, D), 0)
        for n, key in enumerate(state["sel"]):
            base, sub = row_tile(key)
            kv = jnp.full((1, D), key, i32) & -65536
            r = pltpu.bitcast(jnp.where(kv < 0, kv ^ 0x7FFF0000, kv), f32)
            upd = state["y"][n: n + 1] * _sigmoid(r)
            tile = x_tile(base)
            tile = jnp.where(row == sub, tile + upd, tile).astype(bf16)
            for j in range(NT):
                xa32[j, pl.ds(base, 8), :] = _packed(tile[:, 128 * j: 128 * (j + 1)])

    def finish(r0, n, j):
        c, r = divmod(r0, T)
        a = jnp.dot(wide_bf16(ob[c], 0, r, n), _unpacked(wp[3 * NT + j][...]),
                    preferred_element_type=f32)
        b = rows_bf16(xa32, j, r0, n).astype(f32)
        mixed = b + gate[c][pl.ds(r, n), :] * (a - b)
        buf = outb[len(cp_out)]
        bits = _packed(mixed.astype(bf16))
        if len(cp_out) == len(outb) - 1:
            bits = bits | jnp.concatenate([state["clock"] & state["zero"]] * (n // 16), axis=0)
        buf.bitcast(u32)[...] = bits
        cp_out.append(copy(buf, out_hbm.at[pl.ds(r0, n), pl.ds(128 * j, 128)]))
        cp_out[-1].start()

    start(cp_w[0] + cp_x[0] + cp_w[1] + cp_w[2] + cp_vec + cp_x[1] + cp_x[2])
    start(cp_wo + cp_wg + cp_wu + cp_wd)

    fns = dict(
        project=project, finish=finish,
        permute_wqkv=permute_wqkv, permute_wo=permute_wo, permute_x=permute_x,
        scores=scores, softmax=softmax, mix_values=mix_values, router=router,
        select=lambda: select() or gather(), ffn_up=ffn_up, ffn_down=ffn_down, scatter=scatter)
    arrivals = dict(wq=cp_w[0], x0_wk=cp_x[0] + cp_w[1], wv=cp_w[2], x1=cp_vec + cp_x[1],
                    x2_wo=cp_x[2] + cp_wo, ffn=cp_wg + cp_wu + cp_wd)
    zeros[...] = jnp.zeros((8, 128), i32)
    state["zero"] = clock = pltpu.bitcast(jnp.full((8, 128), jnp.max(zeros[...]), i32), u32)
    credit = 0
    for k, (waits, tasks) in enumerate(_schedule()):
        for name in waits:
            wait(arrivals[name])
        if not waits and k % FENCE == 0:
            pl.semaphore_signal(fence, 1)
            pl.semaphore_wait(fence, 1)
        names = [task[0] for task in tasks]
        ticks = (TICK * (names.count("project") + names.count("finish"))
                 - 2 * names.count("softmax") - RT * names.count("router"))
        ticks = max(ticks, 0) / max(names.count("scores") + names.count("mix_values"), 1)
        for name, *args in tasks:
            res = fns[name](*args)
            if res is not None:
                clock = clock ^ pltpu.bitcast(res[-8:], u32)
                credit += ticks
                while credit >= 1:
                    clock = pltpu.roll(clock, 1, 1)
                    credit -= 1
                state["clock"] = clock
    wait(cp_out)


@jax.jit
def pallas_gated_mix__sliding_local_dilated__moe_arch_mod__prompt_kernel(
    A_x: jax.Array,
    A_wqkv: jax.Array,
    A_wo: jax.Array,
    B_x: jax.Array,
    B_w_r: jax.Array,
    B_w_gate: jax.Array,
    B_w_up: jax.Array,
    B_w_down: jax.Array,
    gate_w: jax.Array,
):
    del B_x
    hbm = pl.BlockSpec(memory_space=pltpu.HBM)
    vmem = pltpu.VMEM
    out = pl.pallas_call(
        _kernel,
        in_specs=[hbm] * 8,
        out_specs=hbm,
        out_shape=jax.ShapeDtypeStruct((S, D), bf16),
        scratch_shapes=[
            vmem((NT, S, 128), bf16),
            vmem((3 * NT, D, 128), bf16),
            vmem((NT, D, 128), bf16),
            vmem((NT, F, 128), bf16),
            vmem((NT, F, 128), bf16),
            vmem((NT, F, 128), bf16),
            vmem((D,), bf16),
            vmem((D,), bf16),
            vmem((S // 128, 128), i32),
            [vmem((D, 128), u32)] * 9,
            [vmem((D, 128), f32)] * NT,
            [vmem((D // 2, 128), u32)] * (4 * NT),
            [vmem((NT, T // 2, 128), u32)] * NC,
            [[vmem((NT, T, 128), f32)] + [vmem((NT, HALO + T, 128), f32)] * 2] * NC,
            [vmem((W, T, 128), f32)] * NC,
            [vmem((W, T, 128), f32)] * NC,
            [vmem((NT, T // 2, 128), u32)] * NC,
            [vmem((T, 128), f32)] * NC,
            [vmem((n, 128), bf16) for _, n in OUT_BLOCKS for _ in range(NT)],
            vmem((8, 128), i32),
            pltpu.SemaphoreType.REGULAR,
            pltpu.SemaphoreType.DMA((128,)),
        ],
        compiler_params=pltpu.CompilerParams(vmem_limit_bytes=100 * 1024 * 1024),
    )(A_x.reshape(S, D), A_wqkv, A_wo, B_w_r, B_w_gate.T, B_w_up.T, B_w_down, gate_w)
    return out.reshape(1, S, D)
```

```python
import jax
import jax.numpy as jnp
from jax import lax
import jax.experimental.pallas as pl
import jax.experimental.pallas.tpu as pltpu

S, D, F = 2048, 640, 1728
H, DH, W = 32, 20, 8
NT = D // 128
T = 256
NC = S // T
NI = T // 16
HALO = (W - 1) * 16
SCALE = DH ** -0.5
LOG2E = 1.4426950408889634
KB = ((0, 256), (256, 256), (512, 128))

AN, SN, VN = 16, 128, 16
FP = 128
WO_AT = 3
OUT_BLOCKS = [(r0, T) for r0 in range(0, S, T)]
R, B = 8, 3900
TICK, RT = 3.2, 1
HEAD_ROUTERS = 4
SENDS = (0, 2 * T, 4 * T, 6 * T, 7 * T)
SEND_ROWS = [(a, b - a) for a, b in zip(SENDS, SENDS[1:] + (S,))]
SEND_AT = 2
ARRIVALS = [(38, "wo_x3"), (62, "ffn")]

f32, bf16, u32, i32 = jnp.float32, jnp.bfloat16, jnp.uint32, jnp.int32


def _sigmoid(x):
    return 0.5 * jnp.tanh(0.5 * x) + 0.5


def _packed(x):
    return pltpu.bitcast(x, u32)


def _unpacked(x):
    return pltpu.bitcast(x, bf16)


def _lane_masks(rows):
    lane = lax.broadcasted_iota(i32, (rows, 128), 1)
    lo = lane < 64
    even = (lane & 32) == 0
    mid = (lane >= 32) & (lane < 96)
    return lane, lo, even, mid


def _fold4(p, masks):
    _, lo, even, mid = masks
    c = jnp.where(lo, p[0], p[1]) + pltpu.roll(jnp.where(lo, p[1], p[0]), 64, 1)
    d = jnp.where(mid, p[2], p[3]) + pltpu.roll(jnp.where(mid, p[3], p[2]), 64, 1)
    return jnp.where(even, c, d) + pltpu.roll(jnp.where(even, d, c), 96, 1)


def _spread4(e, masks):
    _, lo, even, mid = masks
    f = pltpu.roll(e, 32, 1)
    c = jnp.where(even, e, f)
    d = jnp.where(even, f, e)
    cr = pltpu.roll(c, 64, 1)
    dr = pltpu.roll(d, 64, 1)
    return [jnp.where(lo, c, cr), jnp.where(lo, cr, c),
            jnp.where(mid, d, dr), jnp.where(mid, dr, d)]


def _interleave(*lists):
    order = sorted(((k + 0.5) / len(l), n, k) for n, l in enumerate(lists) for k in range(len(l)))
    return [lists[n][k] for _, n, k in order]


def _schedule():
    matrix = [(("project", c, n), [("permute_x", c, j) for j in range(NT)])
              for c in range(NC) for n in range(3 * NT)]
    for r0, n in OUT_BLOCKS:
        deps = ([("mix_values", r // T, r % T, VN) for r in range(r0 // T * T, r0 // T * T + T, VN)]
                + [("scatter",)] + [("permute_wo", j) for j in range(NT)])
        matrix += [(("finish", r0, n, j), deps) for j in range(NT)]

    vector = []
    x_data = ["wv_x2"] * 4 + ["wo_x3"] * 4
    for c in range(NC):
        deps = [x_data[c]] + ([("project", c - 2, 3 * NT - 1)] if c > 1 else [])
        vector += [(("permute_x", c, j), 30, deps) for j in range(NT)]
    units = [(f0, min(FP, F - f0)) for f0 in range(0, F, FP)]
    routers = [("router", r0) for r0 in range(0, S, 128)]
    vector += [(t, 500, [x_data[t[1] // T]]) for t in routers]
    vector += [(("select",), 300, routers)]
    ups = [("ffn_up", *u, which) for u in units for which in range(2)]
    vector += [(t, None, [("select",), "ffn"]) for t in ups]
    vector += [(("ffn_down", *u), None, [("ffn_up", *u, 1)]) for u in units]
    vector += [(("scatter",), 100, [("ffn_down", *u) for u in units]
                + [("permute_x", NC - 1, j) for j in range(NT)])]
    for c in range(NC):
        ready = [("project", c, n) for n in range(2 * NT)]
        vector += [(("scores", c, r, AN), 72 * AN // 8, ready) for r in range(0, T, AN)]
        vector += [(("softmax", c, r, SN), 55 * SN // 8,
                    [("scores", c, a, AN) for a in range(r // AN * AN, r + SN, AN)])
                   for r in range(0, T, SN)]
        vector += [(("mix_values", c, r, VN), 78 * VN // 8,
                    [("softmax", c, r // SN * SN, SN), ("project", c, 3 * NT - 1)])
                   for r in range(0, T, VN)]
        if c == WO_AT:
            vector += [(("permute_wo", j), 150, ["wo_x3"]) for j in range(NT)]

    def tiles(c, p):
        return [("project", c, n) for n in range(NT * p, NT * p + NT)]

    def shuffle(p):
        return [("permute_wqkv", p, b) for b in range(len(KB))]

    plan = [(("wq_x0",), shuffle(0) + [("permute_x", 0, j) for j in range(NT)] + tiles(0, 0)),
            (("wk_x1",), [("permute_x", 1, j) for j in range(NT)]
             + _interleave(tiles(1, 0), shuffle(1)) + tiles(0, 1) + tiles(1, 1)),
            (("wv_x2",), shuffle(2) + _interleave(
                tiles(0, 2) + tiles(1, 2), [("permute_x", 2, j) for j in range(NT)],
                [("scores", 0, r, AN) for r in range(0, T, AN)], routers[:HEAD_ROUTERS]))]
    done = [t for waits, tasks in plan for t in list(waits) + tasks]
    matrix = [m for m in matrix if m[0] not in done]
    vector = [v for v in vector if v[0] not in done]
    arrivals, issued = list(ARRIVALS), 6 * NT
    while matrix or vector:
        waits, pieces, budget = (), R, B
        if arrivals and issued >= arrivals[0][0]:
            waits = (arrivals.pop(0)[1],)
        done += list(waits)
        if not vector:
            pieces = len(matrix)
        now = []
        for task, deps in matrix[:pieces]:
            if not all(d in done for d in deps):
                break
            now.append(task)
        picked, small, left = [], [], []
        for item in vector:
            task, cost, deps = item
            ready = all(d in done for d in deps)
            if ready and cost is None and len(small) < max(len(now), 1):
                small.append(task)
            elif ready and cost is not None and cost <= budget:
                picked.append(task)
                budget -= cost
            else:
                left.append(item)
        assert waits or now or small or picked
        plan.append((waits, _interleave(now, small, picked)))
        done += now + small + picked
        issued += len(now)
        matrix, vector = matrix[len(now):], left
    return plan


def _kernel(ax_hbm, wqkv_hbm, wo_hbm, wr_hbm, wg_hbm, wu_hbm, wd_hbm, gw_hbm,
            out_hbm,
            xa, wraw, woraw, wg, wu, wd, wr_ref, gw_ref, rkeys, tmp, tmpf,
            packed, floats, gate, outb, zeros, sems):
    slabs = iter(range(packed.shape[0]))
    wp = [packed.at[next(slabs), pl.ds(0, D // 2), :] for _ in range(4 * NT)]
    xp, ob = ([packed.at[pl.ds(4 * NT + NT * (NC * k + c), NT), pl.ds(0, T // 2), :]
               for c in range(NC)] for k in range(2))
    per_chunk = 3 * NT + 2 * W
    qkv = [[floats.at[pl.ds(per_chunk * c + NT * p, NT)] for p in range(3)] for c in range(NC)]
    logits, probs = ([floats.at[pl.ds(per_chunk * c + 3 * NT + W * k, W)] for c in range(NC)]
                     for k in range(2))
    xa32 = xa.bitcast(u32)
    wraw32, woraw32, wg32, wu32, wd32 = (r.bitcast(u32) for r in (wraw, woraw, wg, wu, wd))

    def rows_bf16(ref32, j, r0, n):
        return _unpacked(ref32[j, pl.ds(r0 // 2, n // 2), :])

    def wide_bf16(ref32, j0, r0, n):
        return jnp.concatenate([rows_bf16(ref32, j0 + j, r0, n) for j in range(NT)], axis=1)

    n_sem = [0]

    def copy(src, dst):
        c = pltpu.make_async_copy(src, dst, sems.at[n_sem[0]])
        n_sem[0] += 1
        return c

    def tiles_in(src, dst, rows, tiles):
        return [copy(src.at[rows, pl.ds(128 * j, 128)], dst.at[j, rows, :]) for j in tiles]

    cp_w = [tiles_in(wqkv_hbm, wraw, pl.ds(0, D), range(NT * p, NT * p + NT)) for p in range(3)]
    x_pieces = ((0, T), (T, T), (2 * T, 2 * T), (4 * T, 4 * T))
    cp_x = [[copy(ax_hbm.at[pl.ds(r0, n), pl.ds(128 * j, 128)], xa.at[j, pl.ds(r0, n), :])
             for j in range(NT)] for (r0, n) in x_pieces]
    cp_wo = tiles_in(wo_hbm, woraw, pl.ds(0, D), range(NT))
    cp_wg = tiles_in(wg_hbm, wg, pl.ds(0, F), range(NT))
    cp_wu = tiles_in(wu_hbm, wu, pl.ds(0, F), range(NT))
    cp_wd = tiles_in(wd_hbm, wd, pl.ds(0, F), range(NT))
    cp_vec = [copy(wr_hbm, wr_ref), copy(gw_hbm, gw_ref)]
    cp_out = [copy(buf, out_hbm.at[pl.ds(r0, n), :]) for buf, (r0, n) in zip(outb, SEND_ROWS)]

    def start(cs):
        for c in cs:
            c.start()

    def wait(cs):
        for c in cs:
            c.wait()

    def permute_wqkv(p, b):
        r0, n = KB[b]
        slot = 3 * p + b
        for j in range(NT):
            w = wraw32[NT * p + j, pl.ds(r0 // 2, n // 2), :]
            if n == 128:
                w = jnp.concatenate([w, jnp.zeros_like(w)], axis=0)
            tmp[slot][pl.ds(128 * j, 128), :] = w.T
        for j in range(NT):
            perm = jnp.concatenate(
                [tmp[slot][pl.ds(d, H, stride=DH), :] for d in range(4 * j, 4 * j + 4)], axis=0)
            wp[NT * p + j][pl.ds(r0 // 2, n // 2), :] = perm.T[: n // 2]

    def permute_wo(j):
        tmpf[j][...] = rows_bf16(woraw32, j, 0, D).astype(f32)
        perm = jnp.concatenate(
            [tmpf[j][pl.ds(d, H, stride=DH), :] for d in range(DH)], axis=0)
        wp[3 * NT + j][...] = _packed(perm.astype(bf16))

    def permute_x(c, j):
        rows = [xa32[j, pl.ds(c * (T // 2) + i, 8, stride=NI), :] for i in range(NI)]
        xp[c][j] = jnp.concatenate(rows, axis=0)

    def project(c, n):
        y = jnp.dot(wide_bf16(xp[c], 0, 0, T), _unpacked(wp[n][...]), preferred_element_type=f32)
        p, j = divmod(n, NT)
        dst = qkv[c][p]
        if p == 0:
            dst[j, pl.ds(0, T), :] = y
            return
        dst[j, pl.ds(HALO, T), :] = y
        row = lax.broadcasted_iota(i32, (8, 128), 0)
        for i in range(NI - (W - 1), NI):
            lo8 = pltpu.roll(y[16 * i: 16 * i + 8], 2, 0)
            hi8 = pltpu.roll(y[16 * i + 8: 16 * i + 16], 2, 0)
            if c > 0:
                prev = pltpu.roll(qkv[c - 1][p][j, pl.ds(HALO + 16 * i + 8, 8), :], 2, 0)
            else:
                prev = jnp.broadcast_to(y[0:1], (8, 128))
            h0 = 16 * (i - (NI - (W - 1)))
            dst[j, pl.ds(h0, 8), :] = jnp.where(row < 2, prev, lo8)
            dst[j, pl.ds(h0 + 8, 8), :] = jnp.where(row < 2, lo8, hi8)

    def window(r0, n):
        rows = range(r0, r0 + n, 16)
        return [(s, [(r, (r - s) // 16) for r in rows if 0 <= r - s <= HALO])
                for s in range(rows[-1], r0 - HALO - 1, -16)]

    def scores(c, r0, n):
        for half in (r0, r0 + 8):
            q = {r: [qkv[c][0][j, pl.ds(r, 8), :] for j in range(NT)]
                 for r in range(half, half + n, 16)}
            for s, users in window(half, n):
                k = [qkv[c][1][j, pl.ds(HALO + s, 8), :] for j in range(NT)]
                for r, w in users:
                    acc = q[r][0] * k[0]
                    for j in range(1, NT):
                        acc = acc + q[r][j] * k[j]
                    logits[c][w, pl.ds(r, 8), :] = acc
        return acc

    def softmax(c, r0, n):
        masks = _lane_masks(n)
        part = [logits[c][w, pl.ds(r0, n), :] for w in range(W)]
        ea, eb = _fold4(part[:4], masks), _fold4(part[4:], masks)
        masked = c == 0 and r0 < HALO
        if masked:
            grp = lax.broadcasted_iota(i32, (n, 128), 1) >> 5
            w_lane = ((grp & 1) << 1) | (grp >> 1)
            row = r0 + lax.broadcasted_iota(i32, (n, 128), 0)
            first = (row & 15) < 2
            ea = jnp.where(first & (w_lane > (row >> 4)), -1e9, ea * SCALE)
            eb = jnp.where(first & (w_lane + 4 > (row >> 4)), -1e9, eb * SCALE)
        m = jnp.maximum(ea, eb)
        m = jnp.maximum(m, pltpu.roll(m, 64, 1))
        m = jnp.maximum(m, pltpu.roll(m, 32, 1))
        cst = LOG2E if masked else SCALE * LOG2E
        ea = jnp.exp2((ea - m) * cst)
        eb = jnp.exp2((eb - m) * cst)
        s = ea + eb
        s = s + pltpu.roll(s, 64, 1)
        s = s + pltpu.roll(s, 32, 1)
        inv = pl.reciprocal(s, approx=True)
        inv = inv * (2.0 - s * inv)
        for w, v in enumerate(_spread4(ea * inv, masks) + _spread4(eb * inv, masks)):
            probs[c][w, pl.ds(r0, n), :] = v

    def mix_values(c, r0, n):
        out = {}
        for half in (r0, r0 + 8):
            prob = {r: [probs[c][w, pl.ds(r, 8), :] for w in range(W)]
                    for r in range(half, half + n, 16)}
            for j in range(NT):
                for s, users in window(half, n):
                    v = qkv[c][2][j, pl.ds(HALO + s, 8), :]
                    for r, w in users:
                        t = prob[r][w] * v
                        out[r, j] = out[r, j] + t if w else t
        for r in range(r0, r0 + n, 16):
            for j in range(NT):
                o = _packed(jnp.concatenate([out[r, j], out[r + 8, j]], axis=0).astype(bf16))
                ob[c][j, pl.ds(r // 16, 8, stride=NI), :] = o
        return o

    def router(r0):
        wr = wr_ref[...].reshape(1, D).astype(f32)
        gw = gw_ref[...].reshape(1, D).astype(f32)
        acc = gacc = None
        for j in range(NT):
            x = rows_bf16(xa32, j, r0, 128).astype(f32)
            t = x * wr[:, 128 * j: 128 * (j + 1)]
            u = x * gw[:, 128 * j: 128 * (j + 1)]
            acc = t if acc is None else acc + t
            gacc = u if gacc is None else gacc + u
        g = _sigmoid(jnp.sum(gacc, axis=1, keepdims=True))
        gate[r0 // T][pl.ds(r0 % T, 128), :] = jnp.broadcast_to(g, (128, 128))
        r = jnp.sum(acc.T, axis=0, keepdims=True)
        r = r.astype(bf16).astype(f32) + 0.0
        bits = pltpu.bitcast(r, i32)
        bits = jnp.where(bits < 0, bits ^ 0x7FFF0000, bits)
        pos = r0 + lax.broadcasted_iota(i32, (1, 128), 1)
        rkeys[pl.ds(r0 // 128, 1), :] = bits | (0xFFFF - pos)

    state = {}

    def select():
        keys = rkeys[...]
        k0 = jnp.max(keys)
        k1 = jnp.max(jnp.where(keys == k0, jnp.iinfo(jnp.int32).min, keys))
        state["sel"] = (k0, k1)

    def row_tile(key):
        idx = jnp.clip(0xFFFF - (key & 0xFFFF), 0, S - 1)
        return pl.multiple_of((idx >> 4) << 3, 8), idx & 15

    def x_tile(base):
        return jnp.concatenate(
            [_unpacked(xa32[j, pl.ds(base, 8), :]) for j in range(NT)], axis=1).astype(f32)

    def gather():
        row = lax.broadcasted_iota(i32, (16, D), 0)
        x_sel = jnp.zeros((16, D), f32)
        for n, key in enumerate(state["sel"]):
            base, sub = row_tile(key)
            picked = jnp.sum(jnp.where(row == sub, x_tile(base), 0.0), axis=0, keepdims=True)
            x_sel = jnp.where(row == n, picked, x_sel)
        state["x_sel"] = x_sel.astype(bf16)

    def ffn_up(f0, n, which):
        w_t = wide_bf16(wu32 if which else wg32, 0, f0, n)
        y = lax.dot_general(state["x_sel"], w_t, (((1,), (1,)), ((), ())),
                            preferred_element_type=f32)
        if which == 0:
            state["g", f0] = y * _sigmoid(y)
        else:
            state["h", f0] = (state["g", f0] * y).astype(bf16)

    def ffn_down(f0, n):
        w = wide_bf16(wd32, 0, f0, n)
        y = jnp.dot(state["h", f0], w, preferred_element_type=f32)
        state["y"] = y if f0 == 0 else state["y"] + y

    def scatter():
        row = lax.broadcasted_iota(i32, (16, D), 0)
        for n, key in enumerate(state["sel"]):
            base, sub = row_tile(key)
            kv = jnp.full((1, D), key, i32) & -65536
            r = pltpu.bitcast(jnp.where(kv < 0, kv ^ 0x7FFF0000, kv), f32)
            upd = state["y"][n: n + 1] * _sigmoid(r)
            tile = x_tile(base)
            tile = jnp.where(row == sub, tile + upd, tile).astype(bf16)
            for j in range(NT):
                xa32[j, pl.ds(base, 8), :] = _packed(tile[:, 128 * j: 128 * (j + 1)])

    def finish(r0, n, j):
        c, r = divmod(r0, T)
        a = jnp.dot(wide_bf16(ob[c], 0, r, n), _unpacked(wp[3 * NT + j][...]),
                    preferred_element_type=f32)
        b = rows_bf16(xa32, j, r0, n).astype(f32)
        mixed = b + gate[c][pl.ds(r, n), :] * (a - b)
        block = max(k for k, start_row in enumerate(SENDS) if start_row <= r0)
        last = r0 + n == S and j == NT - 1
        if last:
            tie = jnp.concatenate([state["clock"] & state["zero"]] * (n // 8), axis=0)
            mixed = pltpu.bitcast(pltpu.bitcast(mixed, u32) | tie, f32)
        outb[block][pl.ds(r0 - SENDS[block], n), pl.ds(128 * j, 128)] = mixed.astype(bf16)
        if block > 0 and r0 == SENDS[block] and j == SEND_AT:
            cp_out[block - 1].start()
        if last:
            cp_out[block].start()

    fns = dict(
        project=project, finish=finish,
        permute_wqkv=permute_wqkv, permute_wo=permute_wo, permute_x=permute_x,
        scores=scores, softmax=softmax, mix_values=mix_values, router=router,
        select=lambda: select() or gather(), ffn_up=ffn_up, ffn_down=ffn_down, scatter=scatter)
    arrivals = dict(wq_x0=cp_w[0] + cp_x[0], wk_x1=cp_w[1] + cp_x[1],
                    wv_x2=cp_w[2] + cp_vec + cp_x[2], wo_x3=cp_x[3] + cp_wo,
                    ffn=cp_wg + cp_wu + cp_wd)
    for copies in arrivals.values():
        start(copies)
    zeros[...] = jnp.zeros((8, 128), i32)
    state["zero"] = clock = pltpu.bitcast(jnp.full((8, 128), jnp.max(zeros[...]), i32), u32)
    credit = 0
    for waits, tasks in _schedule():
        for name in waits:
            wait(arrivals[name])
        names = [task[0] for task in tasks]
        ticks = (TICK * (names.count("project") + names.count("finish"))
                 - 2 * names.count("softmax") - RT * names.count("router"))
        ticks = max(ticks, 0) / max(names.count("scores") + names.count("mix_values"), 1)
        for name, *args in tasks:
            res = fns[name](*args)
            if res is not None:
                clock = clock ^ pltpu.bitcast(res[-8:], u32)
                credit += ticks
                while credit >= 1:
                    clock = pltpu.roll(clock, 1, 1)
                    credit -= 1
                state["clock"] = clock
    wait(cp_out)


@jax.jit
def pallas_gated_mix__sliding_local_dilated__moe_arch_mod__prompt_kernel(
    A_x: jax.Array,
    A_wqkv: jax.Array,
    A_wo: jax.Array,
    B_x: jax.Array,
    B_w_r: jax.Array,
    B_w_gate: jax.Array,
    B_w_up: jax.Array,
    B_w_down: jax.Array,
    gate_w: jax.Array,
):
    del B_x
    hbm = pl.BlockSpec(memory_space=pltpu.HBM)
    vmem = pltpu.VMEM
    out = pl.pallas_call(
        _kernel,
        in_specs=[hbm] * 8,
        out_specs=hbm,
        out_shape=jax.ShapeDtypeStruct((S, D), bf16),
        scratch_shapes=[
            vmem((NT, S, 128), bf16),
            vmem((3 * NT, D, 128), bf16),
            vmem((NT, D, 128), bf16),
            vmem((NT, F, 128), bf16),
            vmem((NT, F, 128), bf16),
            vmem((NT, F, 128), bf16),
            vmem((D,), bf16),
            vmem((D,), bf16),
            vmem((S // 128, 128), i32),
            [vmem((D, 128), u32)] * 9,
            [vmem((D, 128), f32)] * NT,
            vmem((4 * NT + 2 * NC * NT, D // 2, 128), u32),
            vmem((NC * (3 * NT + 2 * W), HALO + T, 128), f32),
            [vmem((T, 128), f32)] * NC,
            [vmem((n, D), bf16) for _, n in SEND_ROWS],
            vmem((8, 128), i32),
            pltpu.SemaphoreType.DMA((128,)),
        ],
        compiler_params=pltpu.CompilerParams(vmem_limit_bytes=100 * 1024 * 1024),
    )(A_x.reshape(S, D), A_wqkv, A_wo, B_w_r, B_w_gate.T, B_w_up.T, B_w_down, gate_w)
    return out.reshape(1, S, D)
```

```python
import jax
import jax.numpy as jnp
from jax import lax
import jax.experimental.pallas as pl
import jax.experimental.pallas.tpu as pltpu

S, D, F = 2048, 640, 1728
H, DH, W = 32, 20, 8
NT = D // 128
T = 256
NC = S // T
NI = T // 16
HALO = (W - 1) * 16
SCALE = DH ** -0.5
LOG2E = 1.4426950408889634
KB = ((0, 256), (256, 256), (512, 128))

AN, SN, VN = 16, 128, 16
FP = 128
WO_AT = 3
OUT_BLOCKS = [(r0, T) for r0 in range(0, S, T)]
R, B = 8, 3650
PM = 128
TICK, RT = 3.2, 1
HEAD_ROUTERS = 4
SENDS = (0, 2 * T, 4 * T, 6 * T, 7 * T)
SEND_ROWS = [(a, b - a) for a, b in zip(SENDS, SENDS[1:] + (S,))]
SEND_AT = 2
ARRIVALS = [(38, "wo_x3"), (62, "ffn")]

f32, bf16, u32, i32 = jnp.float32, jnp.bfloat16, jnp.uint32, jnp.int32


def _sigmoid(x):
    return 0.5 * jnp.tanh(0.5 * x) + 0.5


def _packed(x):
    return pltpu.bitcast(x, u32)


def _unpacked(x):
    return pltpu.bitcast(x, bf16)


def _lane_masks(rows):
    lane = lax.broadcasted_iota(i32, (rows, 128), 1)
    lo = lane < 64
    even = (lane & 32) == 0
    mid = (lane >= 32) & (lane < 96)
    return lane, lo, even, mid


def _fold4(p, masks):
    _, lo, even, mid = masks
    c = jnp.where(lo, p[0], p[1]) + pltpu.roll(jnp.where(lo, p[1], p[0]), 64, 1)
    d = jnp.where(mid, p[2], p[3]) + pltpu.roll(jnp.where(mid, p[3], p[2]), 64, 1)
    return jnp.where(even, c, d) + pltpu.roll(jnp.where(even, d, c), 96, 1)


def _spread4(e, masks):
    _, lo, even, mid = masks
    f = pltpu.roll(e, 32, 1)
    c = jnp.where(even, e, f)
    d = jnp.where(even, f, e)
    cr = pltpu.roll(c, 64, 1)
    dr = pltpu.roll(d, 64, 1)
    return [jnp.where(lo, c, cr), jnp.where(lo, cr, c),
            jnp.where(mid, d, dr), jnp.where(mid, dr, d)]


def _interleave(*lists):
    order = sorted(((k + 0.5) / len(l), n, k) for n, l in enumerate(lists) for k in range(len(l)))
    return [lists[n][k] for _, n, k in order]


def _schedule():
    matrix = [(("project", c, n), [("permute_x", c, j) for j in range(NT)])
              for c in range(NC) for n in range(3 * NT)]
    for r0, n in OUT_BLOCKS:
        deps = ([("mix_values", r // T, r % T, VN) for r in range(r0 // T * T, r0 // T * T + T, VN)]
                + [("scatter",)] + [("permute_wo", j) for j in range(NT)])
        matrix += [(("finish", r0, n, j), deps) for j in range(NT)]

    vector = []
    x_data = ["wv_x2"] * 4 + ["wo_x3"] * 4
    for c in range(NC):
        deps = [x_data[c]] + ([("project", c - 2, 3 * NT - 1)] if c > 1 else [])
        vector += [(("permute_x", c, j), 30, deps) for j in range(NT)]
    units = [(f0, min(FP, F - f0)) for f0 in range(0, F, FP)]
    routers = [("router", r0) for r0 in range(0, S, 128)]
    vector += [(t, 500, [x_data[t[1] // T]]) for t in routers]
    vector += [(("select",), 300, routers)]
    ups = [("ffn_up", *u, which) for u in units for which in range(2)]
    vector += [(t, None, [("select",), "ffn"]) for t in ups]
    vector += [(("ffn_down", *u), None, [("ffn_up", *u, 1)]) for u in units]
    vector += [(("scatter",), 100, [("ffn_down", *u) for u in units]
                + [("permute_x", c, j) for c in range(NC) for j in range(NT)])]
    for c in range(NC):
        ready = [("project", c, n) for n in range(2 * NT)]
        vector += [(("scores", c, r, AN), 72 * AN // 8, ready) for r in range(0, T, AN)]
        vector += [(("softmax", c, r, SN), 55 * SN // 8,
                    [("scores", c, a, AN) for a in range(r // AN * AN, r + SN, AN)])
                   for r in range(0, T, SN)]
        vector += [(("mix_values", c, r, VN), 78 * VN // 8,
                    [("softmax", c, r // SN * SN, SN), ("project", c, 3 * NT - 1)])
                   for r in range(0, T, VN)]
        if c == WO_AT:
            vector += [(("permute_wo", j), 150, ["wo_x3"]) for j in range(NT)]

    def tiles(c, p):
        return [("project", c, n) for n in range(NT * p, NT * p + NT)]

    def shuffle(p):
        return [("permute_wqkv", p, b) for b in range(len(KB))]

    plan = [(("wq_x0",), shuffle(0) + [("permute_x", 0, j) for j in range(NT)] + tiles(0, 0)),
            (("wk_x1",), [("permute_x", 1, j) for j in range(NT)]
             + _interleave(tiles(1, 0), shuffle(1)) + tiles(0, 1) + tiles(1, 1)),
            (("wv_x2",), shuffle(2) + _interleave(
                tiles(0, 2) + tiles(1, 2), [("permute_x", 2, j) for j in range(NT)],
                [("scores", 0, r, AN) for r in range(0, T, AN)], routers[:HEAD_ROUTERS]))]
    done = [t for waits, tasks in plan for t in list(waits) + tasks]
    matrix = [m for m in matrix if m[0] not in done]
    vector = [v for v in vector if v[0] not in done]
    arrivals, issued = list(ARRIVALS), 6 * NT
    while matrix or vector:
        waits, pieces, budget = (), R, B
        if arrivals and issued >= arrivals[0][0]:
            waits = (arrivals.pop(0)[1],)
        done += list(waits)
        if not vector:
            pieces = len(matrix)
        now = []
        for task, deps in matrix[:pieces]:
            if not all(d in done for d in deps):
                break
            now.append(task)
        picked, small, left = [], [], []
        for item in vector:
            task, cost, deps = item
            ready = all(d in done for d in deps)
            if ready and cost is None and len(small) < max(len(now), 1):
                small.append(task)
            elif ready and cost is not None and cost <= budget:
                picked.append(task)
                budget -= cost
            else:
                left.append(item)
        assert waits or now or small or picked
        plan.append((waits, _interleave(now, small, picked)))
        done += now + small + picked
        issued += len(now)
        matrix, vector = matrix[len(now):], left
    return plan


def _kernel(ax_hbm, wqkv_hbm, wo_hbm, wr_hbm, wg_hbm, wu_hbm, wd_hbm, gw_hbm,
            out_hbm,
            xa, wraw, woraw, wg, wu, wd, wr_ref, gw_ref, rkeys, tmp, tmpf,
            packed, floats, gate, outb, zeros, sems):
    slabs = iter(range(packed.shape[0]))
    wp = [packed.at[next(slabs), pl.ds(0, D // 2), :] for _ in range(4 * NT)]
    xp, ob = ([packed.at[pl.ds(4 * NT + NT * (NC * k + c), NT), pl.ds(0, T // 2), :]
               for c in range(NC)] for k in range(2))
    per_chunk = 3 * NT + 2 * W
    qkv = [[floats.at[pl.ds(per_chunk * c + NT * p, NT)] for p in range(3)] for c in range(NC)]
    logits, probs = ([floats.at[pl.ds(per_chunk * c + 3 * NT + W * k, W)] for c in range(NC)]
                     for k in range(2))
    xa32 = xa.bitcast(u32)
    wraw32, woraw32, wg32, wu32, wd32 = (r.bitcast(u32) for r in (wraw, woraw, wg, wu, wd))

    def rows_bf16(ref32, j, r0, n):
        return _unpacked(ref32[j, pl.ds(r0 // 2, n // 2), :])

    def wide_bf16(ref32, j0, r0, n):
        return jnp.concatenate([rows_bf16(ref32, j0 + j, r0, n) for j in range(NT)], axis=1)

    n_sem = [0]

    def copy(src, dst):
        c = pltpu.make_async_copy(src, dst, sems.at[n_sem[0]])
        n_sem[0] += 1
        return c

    def tiles_in(src, dst, rows, tiles):
        return [copy(src.at[rows, pl.ds(128 * j, 128)], dst.at[j, rows, :]) for j in tiles]

    cp_w = [tiles_in(wqkv_hbm, wraw, pl.ds(0, D), range(NT * p, NT * p + NT)) for p in range(3)]
    x_pieces = ((0, T), (T, T), (2 * T, 2 * T), (4 * T, 4 * T))
    cp_x = [[copy(ax_hbm.at[pl.ds(r0, n), pl.ds(128 * j, 128)], xa.at[j, pl.ds(r0, n), :])
             for j in range(NT)] for (r0, n) in x_pieces]
    cp_wo = tiles_in(wo_hbm, woraw, pl.ds(0, D), range(NT))
    cp_wg = tiles_in(wg_hbm, wg, pl.ds(0, F), range(NT))
    cp_wu = tiles_in(wu_hbm, wu, pl.ds(0, F), range(NT))
    cp_wd = tiles_in(wd_hbm, wd, pl.ds(0, F), range(NT))
    cp_vec = [copy(wr_hbm, wr_ref), copy(gw_hbm, gw_ref)]
    cp_out = [copy(buf, out_hbm.at[pl.ds(r0, n), :]) for buf, (r0, n) in zip(outb, SEND_ROWS)]

    def start(cs):
        for c in cs:
            c.start()

    def wait(cs):
        for c in cs:
            c.wait()

    def permute_wqkv(p, b):
        r0, n = KB[b]
        slot = 3 * p + b
        for j in range(NT):
            w = wraw32[NT * p + j, pl.ds(r0 // 2, n // 2), :]
            if n == 128:
                w = jnp.concatenate([w, jnp.zeros_like(w)], axis=0)
            tmp[slot][pl.ds(128 * j, 128), :] = w.T
        for j in range(NT):
            perm = jnp.concatenate(
                [tmp[slot][pl.ds(d, H, stride=DH), :] for d in range(4 * j, 4 * j + 4)], axis=0)
            wp[NT * p + j][pl.ds(r0 // 2, n // 2), :] = perm.T[: n // 2]

    def permute_wo(j):
        tmpf[j][...] = rows_bf16(woraw32, j, 0, D).astype(f32)
        perm = jnp.concatenate(
            [tmpf[j][pl.ds(d, H, stride=DH), :] for d in range(DH)], axis=0)
        wp[3 * NT + j][...] = _packed(perm.astype(bf16))

    def permute_x(c, j):
        rows = [xa32[j, pl.ds(c * (T // 2) + i, 8, stride=NI), :] for i in range(NI)]
        xp[c][j] = jnp.concatenate(rows, axis=0)

    def matmul(lhs, r0, n, tile):
        return jnp.concatenate(
            [jnp.dot(wide_bf16(lhs, 0, m, PM), _unpacked(wp[tile][...]), preferred_element_type=f32)
             for m in range(r0, r0 + n, PM)], axis=0)

    def project(c, n):
        y = matmul(xp[c], 0, T, n)
        p, j = divmod(n, NT)
        dst = qkv[c][p]
        if p == 0:
            dst[j, pl.ds(0, T), :] = y
            return
        dst[j, pl.ds(HALO, T), :] = y
        row = lax.broadcasted_iota(i32, (8, 128), 0)
        for i in range(NI - (W - 1), NI):
            lo8 = pltpu.roll(y[16 * i: 16 * i + 8], 2, 0)
            hi8 = pltpu.roll(y[16 * i + 8: 16 * i + 16], 2, 0)
            if c > 0:
                prev = pltpu.roll(qkv[c - 1][p][j, pl.ds(HALO + 16 * i + 8, 8), :], 2, 0)
            else:
                prev = jnp.broadcast_to(y[0:1], (8, 128))
            h0 = 16 * (i - (NI - (W - 1)))
            dst[j, pl.ds(h0, 8), :] = jnp.where(row < 2, prev, lo8)
            dst[j, pl.ds(h0 + 8, 8), :] = jnp.where(row < 2, lo8, hi8)

    def window(r0, n):
        rows = range(r0, r0 + n, 16)
        return [(s, [(r, (r - s) // 16) for r in rows if 0 <= r - s <= HALO])
                for s in range(rows[-1], r0 - HALO - 1, -16)]

    def scores(c, r0, n):
        for half in (r0, r0 + 8):
            q = {r: [qkv[c][0][j, pl.ds(r, 8), :] for j in range(NT)]
                 for r in range(half, half + n, 16)}
            for s, users in window(half, n):
                k = [qkv[c][1][j, pl.ds(HALO + s, 8), :] for j in range(NT)]
                for r, w in users:
                    acc = q[r][0] * k[0]
                    for j in range(1, NT):
                        acc = acc + q[r][j] * k[j]
                    logits[c][w, pl.ds(r, 8), :] = acc
        return acc

    def softmax(c, r0, n):
        masks = _lane_masks(n)
        part = [logits[c][w, pl.ds(r0, n), :] for w in range(W)]
        ea, eb = _fold4(part[:4], masks), _fold4(part[4:], masks)
        masked = c == 0 and r0 < HALO
        if masked:
            grp = lax.broadcasted_iota(i32, (n, 128), 1) >> 5
            w_lane = ((grp & 1) << 1) | (grp >> 1)
            row = r0 + lax.broadcasted_iota(i32, (n, 128), 0)
            first = (row & 15) < 2
            ea = jnp.where(first & (w_lane > (row >> 4)), -1e9, ea * SCALE)
            eb = jnp.where(first & (w_lane + 4 > (row >> 4)), -1e9, eb * SCALE)
        m = jnp.maximum(ea, eb)
        m = jnp.maximum(m, pltpu.roll(m, 64, 1))
        m = jnp.maximum(m, pltpu.roll(m, 32, 1))
        cst = LOG2E if masked else SCALE * LOG2E
        ea = jnp.exp2((ea - m) * cst)
        eb = jnp.exp2((eb - m) * cst)
        s = ea + eb
        s = s + pltpu.roll(s, 64, 1)
        s = s + pltpu.roll(s, 32, 1)
        inv = pl.reciprocal(s, approx=True)
        inv = inv * (2.0 - s * inv)
        for w, v in enumerate(_spread4(ea * inv, masks) + _spread4(eb * inv, masks)):
            probs[c][w, pl.ds(r0, n), :] = v

    def mix_values(c, r0, n):
        out = {}
        for half in (r0, r0 + 8):
            prob = {r: [probs[c][w, pl.ds(r, 8), :] for w in range(W)]
                    for r in range(half, half + n, 16)}
            for j in range(NT):
                for s, users in window(half, n):
                    v = qkv[c][2][j, pl.ds(HALO + s, 8), :]
                    for r, w in users:
                        t = prob[r][w] * v
                        out[r, j] = out[r, j] + t if w else t
        for r in range(r0, r0 + n, 16):
            for j in range(NT):
                o = _packed(jnp.concatenate([out[r, j], out[r + 8, j]], axis=0).astype(bf16))
                ob[c][j, pl.ds(r // 16, 8, stride=NI), :] = o
        return o

    def router(r0):
        wr = wr_ref[...].reshape(1, D).astype(f32)
        gw = gw_ref[...].reshape(1, D).astype(f32)
        acc = gacc = None
        for j in range(NT):
            x = rows_bf16(xa32, j, r0, 128).astype(f32)
            t = x * wr[:, 128 * j: 128 * (j + 1)]
            u = x * gw[:, 128 * j: 128 * (j + 1)]
            acc = t if acc is None else acc + t
            gacc = u if gacc is None else gacc + u
        g = _sigmoid(jnp.sum(gacc, axis=1, keepdims=True))
        gate[r0 // T][pl.ds(r0 % T, 128), :] = jnp.broadcast_to(g, (128, 128))
        r = jnp.sum(acc.T, axis=0, keepdims=True)
        r = r.astype(bf16).astype(f32) + 0.0
        bits = pltpu.bitcast(r, i32)
        bits = jnp.where(bits < 0, bits ^ 0x7FFF0000, bits)
        pos = r0 + lax.broadcasted_iota(i32, (1, 128), 1)
        rkeys[pl.ds(r0 // 128, 1), :] = bits | (0xFFFF - pos)

    state = {}

    def select():
        keys = rkeys[...]
        k0 = jnp.max(keys)
        k1 = jnp.max(jnp.where(keys == k0, jnp.iinfo(jnp.int32).min, keys))
        state["sel"] = (k0, k1)

    def row_tile(key):
        idx = jnp.clip(0xFFFF - (key & 0xFFFF), 0, S - 1)
        return pl.multiple_of((idx >> 4) << 3, 8), idx & 15

    def x_tile(base):
        return jnp.concatenate(
            [_unpacked(xa32[j, pl.ds(base, 8), :]) for j in range(NT)], axis=1).astype(f32)

    def gather():
        row = lax.broadcasted_iota(i32, (16, D), 0)
        x_sel = jnp.zeros((16, D), f32)
        for n, key in enumerate(state["sel"]):
            base, sub = row_tile(key)
            picked = jnp.sum(jnp.where(row == sub, x_tile(base), 0.0), axis=0, keepdims=True)
            x_sel = jnp.where(row == n, picked, x_sel)
        state["x_sel"] = x_sel.astype(bf16)

    def ffn_up(f0, n, which):
        w_t = wide_bf16(wu32 if which else wg32, 0, f0, n)
        y = lax.dot_general(state["x_sel"], w_t, (((1,), (1,)), ((), ())),
                            preferred_element_type=f32)
        if which == 0:
            state["g", f0] = y * _sigmoid(y)
        else:
            state["h", f0] = (state["g", f0] * y).astype(bf16)

    def ffn_down(f0, n):
        w = wide_bf16(wd32, 0, f0, n)
        y = jnp.dot(state["h", f0], w, preferred_element_type=f32)
        state["y"] = y if f0 == 0 else state["y"] + y

    def scatter():
        row = lax.broadcasted_iota(i32, (16, D), 0)
        for n, key in enumerate(state["sel"]):
            base, sub = row_tile(key)
            kv = jnp.full((1, D), key, i32) & -65536
            r = pltpu.bitcast(jnp.where(kv < 0, kv ^ 0x7FFF0000, kv), f32)
            upd = state["y"][n: n + 1] * _sigmoid(r)
            tile = x_tile(base)
            tile = jnp.where(row == sub, tile + upd, tile).astype(bf16)
            for j in range(NT):
                xa32[j, pl.ds(base, 8), :] = _packed(tile[:, 128 * j: 128 * (j + 1)])

    def finish(r0, n, j):
        c, r = divmod(r0, T)
        a = matmul(ob[c], r, n, 3 * NT + j)
        b = rows_bf16(xa32, j, r0, n).astype(f32)
        mixed = b + gate[c][pl.ds(r, n), :] * (a - b)
        block = max(k for k, start_row in enumerate(SENDS) if start_row <= r0)
        last = r0 + n == S and j == NT - 1
        if last:
            tie = jnp.concatenate([state["clock"] & state["zero"]] * (n // 8), axis=0)
            mixed = pltpu.bitcast(pltpu.bitcast(mixed, u32) | tie, f32)
        outb[block][pl.ds(r0 - SENDS[block], n), pl.ds(128 * j, 128)] = mixed.astype(bf16)
        if block > 0 and r0 == SENDS[block] and j == SEND_AT:
            cp_out[block - 1].start()
        if last:
            cp_out[block].start()

    fns = dict(
        project=project, finish=finish,
        permute_wqkv=permute_wqkv, permute_wo=permute_wo, permute_x=permute_x,
        scores=scores, softmax=softmax, mix_values=mix_values, router=router,
        select=lambda: select() or gather(), ffn_up=ffn_up, ffn_down=ffn_down, scatter=scatter)
    arrivals = dict(wq_x0=cp_w[0] + cp_x[0], wk_x1=cp_w[1] + cp_x[1],
                    wv_x2=cp_w[2] + cp_vec + cp_x[2], wo_x3=cp_x[3] + cp_wo,
                    ffn=cp_wg + cp_wu + cp_wd)
    for copies in arrivals.values():
        start(copies)
    zeros[...] = jnp.zeros((8, 128), i32)
    state["zero"] = clock = pltpu.bitcast(jnp.full((8, 128), jnp.max(zeros[...]), i32), u32)
    credit = 0
    for waits, tasks in _schedule():
        for name in waits:
            wait(arrivals[name])
        names = [task[0] for task in tasks]
        ticks = (TICK * (names.count("project") + names.count("finish"))
                 - 2 * names.count("softmax") - RT * names.count("router"))
        ticks = max(ticks, 0) / max(names.count("scores") + names.count("mix_values"), 1)
        for name, *args in tasks:
            res = fns[name](*args)
            if res is not None:
                clock = clock ^ pltpu.bitcast(res[-8:], u32)
                credit += ticks
                while credit >= 1:
                    clock = pltpu.roll(clock, 1, 1)
                    credit -= 1
                state["clock"] = clock
    wait(cp_out)


@jax.jit
def pallas_gated_mix__sliding_local_dilated__moe_arch_mod__prompt_kernel(
    A_x: jax.Array,
    A_wqkv: jax.Array,
    A_wo: jax.Array,
    B_x: jax.Array,
    B_w_r: jax.Array,
    B_w_gate: jax.Array,
    B_w_up: jax.Array,
    B_w_down: jax.Array,
    gate_w: jax.Array,
):
    del B_x
    hbm = pl.BlockSpec(memory_space=pltpu.HBM)
    vmem = pltpu.VMEM
    out = pl.pallas_call(
        _kernel,
        in_specs=[hbm] * 8,
        out_specs=hbm,
        out_shape=jax.ShapeDtypeStruct((S, D), bf16),
        scratch_shapes=[
            vmem((NT, S, 128), bf16),
            vmem((3 * NT, D, 128), bf16),
            vmem((NT, D, 128), bf16),
            vmem((NT, F, 128), bf16),
            vmem((NT, F, 128), bf16),
            vmem((NT, F, 128), bf16),
            vmem((D,), bf16),
            vmem((D,), bf16),
            vmem((S // 128, 128), i32),
            [vmem((D, 128), u32)] * 9,
            [vmem((D, 128), f32)] * NT,
            vmem((4 * NT + 2 * NC * NT, D // 2, 128), u32),
            vmem((NC * (3 * NT + 2 * W), HALO + T, 128), f32),
            [vmem((T, 128), f32)] * NC,
            [vmem((n, D), bf16) for _, n in SEND_ROWS],
            vmem((8, 128), i32),
            pltpu.SemaphoreType.DMA((128,)),
        ],
        compiler_params=pltpu.CompilerParams(vmem_limit_bytes=100 * 1024 * 1024),
    )(A_x.reshape(S, D), A_wqkv, A_wo, B_w_r, B_w_gate.T, B_w_up.T, B_w_down, gate_w)
    return out.reshape(1, S, D)
```

```python
import jax
import jax.numpy as jnp
from jax import lax
import jax.experimental.pallas as pl
import jax.experimental.pallas.tpu as pltpu

S, D, F = 2048, 640, 1728
H, DH, W = 32, 20, 8
NT = D // 128
T = 256
NC = S // T
NI = T // 16
HALO = (W - 1) * 16
SCALE = DH ** -0.5
LOG2E = 1.4426950408889634
KB = ((0, 256), (256, 256), (512, 128))

AN, SN, VN = 16, 128, 16
FP = 128
WO_AT = 3
OUT_BLOCKS = [(r0, T) for r0 in range(0, S, T)]
R, B = 8, 3650
PM = 128
TICK, RT = 3.2, 1
HEAD_ROUTERS = 2
SENDS = (0, 2 * T, 4 * T, 6 * T, 7 * T)
SEND_ROWS = [(a, b - a) for a, b in zip(SENDS, SENDS[1:] + (S,))]
SEND_AT = 2
ARRIVALS = [(38, "wo_x3"), (62, "ffn"), (78, "wd")]

f32, bf16, u32, i32 = jnp.float32, jnp.bfloat16, jnp.uint32, jnp.int32


def _sigmoid(x):
    return 0.5 * jnp.tanh(0.5 * x) + 0.5


def _packed(x):
    return pltpu.bitcast(x, u32)


def _unpacked(x):
    return pltpu.bitcast(x, bf16)


def _lane_masks(rows):
    lane = lax.broadcasted_iota(i32, (rows, 128), 1)
    lo = lane < 64
    even = (lane & 32) == 0
    mid = (lane >= 32) & (lane < 96)
    return lane, lo, even, mid


def _fold4(p, masks):
    _, lo, even, mid = masks
    c = jnp.where(lo, p[0], p[1]) + pltpu.roll(jnp.where(lo, p[1], p[0]), 64, 1)
    d = jnp.where(mid, p[2], p[3]) + pltpu.roll(jnp.where(mid, p[3], p[2]), 64, 1)
    return jnp.where(even, c, d) + pltpu.roll(jnp.where(even, d, c), 96, 1)


def _spread4(e, masks):
    _, lo, even, mid = masks
    f = pltpu.roll(e, 32, 1)
    c = jnp.where(even, e, f)
    d = jnp.where(even, f, e)
    cr = pltpu.roll(c, 64, 1)
    dr = pltpu.roll(d, 64, 1)
    return [jnp.where(lo, c, cr), jnp.where(lo, cr, c),
            jnp.where(mid, d, dr), jnp.where(mid, dr, d)]


def _interleave(*lists):
    order = sorted(((k + 0.5) / len(l), n, k) for n, l in enumerate(lists) for k in range(len(l)))
    return [lists[n][k] for _, n, k in order]


def _schedule():
    matrix = [(("project", c, n), [("permute_x", c, j) for j in range(NT)])
              for c in range(NC) for n in range(3 * NT)]
    for r0, n in OUT_BLOCKS:
        deps = ([("mix_values", r // T, r % T, VN) for r in range(r0 // T * T, r0 // T * T + T, VN)]
                + [("scatter",)] + [("permute_wo", j) for j in range(NT)])
        matrix += [(("finish", r0, n, j), deps) for j in range(NT)]

    vector = []
    x_data = ["wv_x2"] * 4 + ["wo_x3"] * 4
    for c in range(NC):
        deps = [x_data[c]] + ([("project", c - 2, 3 * NT - 1)] if c > 1 else [])
        vector += [(("permute_x", c, j), 30, deps) for j in range(NT)]
    units = [(f0, min(FP, F - f0)) for f0 in range(0, F, FP)]
    routers = [("router", r0) for r0 in range(0, S, 128)]
    vector += [(t, 500, [x_data[t[1] // T]]) for t in routers]
    vector += [(("select",), 300, routers)]
    ups = [("ffn_up", *u, which) for u in units for which in range(2)]
    vector += [(t, None, [("select",), "ffn"]) for t in ups]
    vector += [(("ffn_down", *u), None, [("ffn_up", *u, 1), "wd"]) for u in units]
    vector += [(("scatter",), 100, [("ffn_down", *u) for u in units]
                + [("permute_x", c, j) for c in range(NC) for j in range(NT)])]
    for c in range(NC):
        ready = [("project", c, n) for n in range(2 * NT)]
        vector += [(("scores", c, r, AN), 72 * AN // 8, ready) for r in range(0, T, AN)]
        vector += [(("softmax", c, r, SN), 55 * SN // 8,
                    [("scores", c, a, AN) for a in range(r // AN * AN, r + SN, AN)])
                   for r in range(0, T, SN)]
        vector += [(("mix_values", c, r, VN), 78 * VN // 8,
                    [("softmax", c, r // SN * SN, SN), ("project", c, 3 * NT - 1)])
                   for r in range(0, T, VN)]
        if c == WO_AT:
            vector += [(("permute_wo", j), 150, ["wo_x3"]) for j in range(NT)]

    def tiles(c, p):
        return [("project", c, n) for n in range(NT * p, NT * p + NT)]

    def shuffle(p):
        return [("permute_wqkv", p, b) for b in range(len(KB))]

    plan = [(("wq_x0",), shuffle(0) + [("permute_x", 0, j) for j in range(NT)] + tiles(0, 0)),
            (("wk_x1",), [("permute_x", 1, j) for j in range(NT)]
             + _interleave(tiles(1, 0), shuffle(1)) + tiles(0, 1) + tiles(1, 1)),
            (("wv_x2",), shuffle(2) + _interleave(
                tiles(0, 2) + tiles(1, 2), [("permute_x", 2, j) for j in range(NT)],
                [("scores", 0, r, AN) for r in range(0, T, AN)], routers[:HEAD_ROUTERS]))]
    done = [t for waits, tasks in plan for t in list(waits) + tasks]
    matrix = [m for m in matrix if m[0] not in done]
    vector = [v for v in vector if v[0] not in done]
    arrivals, issued = list(ARRIVALS), 6 * NT
    while matrix or vector:
        waits, pieces, budget = (), R, B
        if arrivals and issued >= arrivals[0][0]:
            waits = (arrivals.pop(0)[1],)
        done += list(waits)
        if not vector:
            pieces = len(matrix)
        now = []
        for task, deps in matrix[:pieces]:
            if not all(d in done for d in deps):
                break
            now.append(task)
        picked, small, left = [], [], []
        for item in vector:
            task, cost, deps = item
            ready = all(d in done for d in deps)
            if ready and cost is None and len(small) < max(len(now), 1):
                small.append(task)
            elif ready and cost is not None and cost <= budget:
                picked.append(task)
                budget -= cost
            else:
                left.append(item)
        assert waits or now or small or picked
        plan.append((waits, _interleave(now, small, picked)))
        done += now + small + picked
        issued += len(now)
        matrix, vector = matrix[len(now):], left
    return plan


def _kernel(ax_hbm, wqkv_hbm, wo_hbm, wr_hbm, wg_hbm, wu_hbm, wd_hbm, gw_hbm,
            out_hbm,
            xa, wraw, woraw, wg, wu, wd, wr_ref, gw_ref, rkeys, tmp, tmpf,
            packed, floats, gate, outb, zeros, sems):
    slabs = iter(range(packed.shape[0]))
    wp = [packed.at[next(slabs), pl.ds(0, D // 2), :] for _ in range(4 * NT)]
    xp, ob = ([packed.at[pl.ds(4 * NT + NT * (NC * k + c), NT), pl.ds(0, T // 2), :]
               for c in range(NC)] for k in range(2))
    per_chunk = 3 * NT + 2 * W
    qkv = [[floats.at[pl.ds(per_chunk * c + NT * p, NT)] for p in range(3)] for c in range(NC)]
    logits, probs = ([floats.at[pl.ds(per_chunk * c + 3 * NT + W * k, W)] for c in range(NC)]
                     for k in range(2))
    xa32 = xa.bitcast(u32)
    wraw32, woraw32, wg32, wu32, wd32 = (r.bitcast(u32) for r in (wraw, woraw, wg, wu, wd))

    def rows_bf16(ref32, j, r0, n):
        return _unpacked(ref32[j, pl.ds(r0 // 2, n // 2), :])

    def wide_bf16(ref32, j0, r0, n):
        return jnp.concatenate([rows_bf16(ref32, j0 + j, r0, n) for j in range(NT)], axis=1)

    n_sem = [0]

    def copy(src, dst):
        c = pltpu.make_async_copy(src, dst, sems.at[n_sem[0]])
        n_sem[0] += 1
        return c

    def tiles_in(src, dst, rows, tiles):
        return [copy(src.at[rows, pl.ds(128 * j, 128)], dst.at[j, rows, :]) for j in tiles]

    cp_w = [tiles_in(wqkv_hbm, wraw, pl.ds(0, D), range(NT * p, NT * p + NT)) for p in range(3)]
    x_pieces = ((0, T), (T, T), (2 * T, 2 * T), (4 * T, 4 * T))
    cp_x = [[copy(ax_hbm.at[pl.ds(r0, n), pl.ds(128 * j, 128)], xa.at[j, pl.ds(r0, n), :])
             for j in range(NT)] for (r0, n) in x_pieces]
    cp_wo = tiles_in(wo_hbm, woraw, pl.ds(0, D), range(NT))
    cp_wg = tiles_in(wg_hbm, wg, pl.ds(0, F), range(NT))
    cp_wu = tiles_in(wu_hbm, wu, pl.ds(0, F), range(NT))
    cp_wd = tiles_in(wd_hbm, wd, pl.ds(0, F), range(NT))
    cp_vec = [copy(wr_hbm, wr_ref), copy(gw_hbm, gw_ref)]
    cp_out = [copy(buf, out_hbm.at[pl.ds(r0, n), :]) for buf, (r0, n) in zip(outb, SEND_ROWS)]

    def start(cs):
        for c in cs:
            c.start()

    def wait(cs):
        for c in cs:
            c.wait()

    def permute_wqkv(p, b):
        r0, n = KB[b]
        slot = 3 * p + b
        for j in range(NT):
            w = wraw32[NT * p + j, pl.ds(r0 // 2, n // 2), :]
            if n == 128:
                w = jnp.concatenate([w, jnp.zeros_like(w)], axis=0)
            tmp[slot][pl.ds(128 * j, 128), :] = w.T
        for j in range(NT):
            perm = jnp.concatenate(
                [tmp[slot][pl.ds(d, H, stride=DH), :] for d in range(4 * j, 4 * j + 4)], axis=0)
            wp[NT * p + j][pl.ds(r0 // 2, n // 2), :] = perm.T[: n // 2]

    def permute_wo(j):
        tmpf[j][...] = rows_bf16(woraw32, j, 0, D).astype(f32)
        perm = jnp.concatenate(
            [tmpf[j][pl.ds(d, H, stride=DH), :] for d in range(DH)], axis=0)
        wp[3 * NT + j][...] = _packed(perm.astype(bf16))

    def permute_x(c, j):
        rows = [xa32[j, pl.ds(c * (T // 2) + i, 8, stride=NI), :] for i in range(NI)]
        xp[c][j] = jnp.concatenate(rows, axis=0)

    def matmul(lhs, r0, n, tile):
        return jnp.concatenate(
            [jnp.dot(wide_bf16(lhs, 0, m, PM), _unpacked(wp[tile][...]), preferred_element_type=f32)
             for m in range(r0, r0 + n, PM)], axis=0)

    def project(c, n):
        y = matmul(xp[c], 0, T, n)
        p, j = divmod(n, NT)
        dst = qkv[c][p]
        if p == 0:
            dst[j, pl.ds(0, T), :] = y
            return
        dst[j, pl.ds(HALO, T), :] = y
        row = lax.broadcasted_iota(i32, (8, 128), 0)
        for i in range(NI - (W - 1), NI):
            lo8 = pltpu.roll(y[16 * i: 16 * i + 8], 2, 0)
            hi8 = pltpu.roll(y[16 * i + 8: 16 * i + 16], 2, 0)
            if c > 0:
                prev = pltpu.roll(qkv[c - 1][p][j, pl.ds(HALO + 16 * i + 8, 8), :], 2, 0)
            else:
                prev = jnp.broadcast_to(y[0:1], (8, 128))
            h0 = 16 * (i - (NI - (W - 1)))
            dst[j, pl.ds(h0, 8), :] = jnp.where(row < 2, prev, lo8)
            dst[j, pl.ds(h0 + 8, 8), :] = jnp.where(row < 2, lo8, hi8)

    def window(r0, n):
        rows = range(r0, r0 + n, 16)
        return [(s, [(r, (r - s) // 16) for r in rows if 0 <= r - s <= HALO])
                for s in range(rows[-1], r0 - HALO - 1, -16)]

    def scores(c, r0, n):
        for half in (r0, r0 + 8):
            q = {r: [qkv[c][0][j, pl.ds(r, 8), :] for j in range(NT)]
                 for r in range(half, half + n, 16)}
            for s, users in window(half, n):
                k = [qkv[c][1][j, pl.ds(HALO + s, 8), :] for j in range(NT)]
                for r, w in users:
                    acc = q[r][0] * k[0]
                    for j in range(1, NT):
                        acc = acc + q[r][j] * k[j]
                    logits[c][w, pl.ds(r, 8), :] = acc
        return acc

    def softmax(c, r0, n):
        masks = _lane_masks(n)
        part = [logits[c][w, pl.ds(r0, n), :] for w in range(W)]
        ea, eb = _fold4(part[:4], masks), _fold4(part[4:], masks)
        masked = c == 0 and r0 < HALO
        if masked:
            grp = lax.broadcasted_iota(i32, (n, 128), 1) >> 5
            w_lane = ((grp & 1) << 1) | (grp >> 1)
            row = r0 + lax.broadcasted_iota(i32, (n, 128), 0)
            first = (row & 15) < 2
            ea = jnp.where(first & (w_lane > (row >> 4)), -1e9, ea * SCALE)
            eb = jnp.where(first & (w_lane + 4 > (row >> 4)), -1e9, eb * SCALE)
        m = jnp.maximum(ea, eb)
        m = jnp.maximum(m, pltpu.roll(m, 64, 1))
        m = jnp.maximum(m, pltpu.roll(m, 32, 1))
        cst = LOG2E if masked else SCALE * LOG2E
        ea = jnp.exp2((ea - m) * cst)
        eb = jnp.exp2((eb - m) * cst)
        s = ea + eb
        s = s + pltpu.roll(s, 64, 1)
        s = s + pltpu.roll(s, 32, 1)
        inv = pl.reciprocal(s, approx=True)
        inv = inv * (2.0 - s * inv)
        for w, v in enumerate(_spread4(ea * inv, masks) + _spread4(eb * inv, masks)):
            probs[c][w, pl.ds(r0, n), :] = v

    def mix_values(c, r0, n):
        out = {}
        for half in (r0, r0 + 8):
            prob = {r: [probs[c][w, pl.ds(r, 8), :] for w in range(W)]
                    for r in range(half, half + n, 16)}
            for j in range(NT):
                for s, users in window(half, n):
                    v = qkv[c][2][j, pl.ds(HALO + s, 8), :]
                    for r, w in users:
                        t = prob[r][w] * v
                        out[r, j] = out[r, j] + t if w else t
        for r in range(r0, r0 + n, 16):
            for j in range(NT):
                o = _packed(jnp.concatenate([out[r, j], out[r + 8, j]], axis=0).astype(bf16))
                ob[c][j, pl.ds(r // 16, 8, stride=NI), :] = o
        return o

    def router(r0):
        wr = wr_ref[...].reshape(1, D).astype(f32)
        gw = gw_ref[...].reshape(1, D).astype(f32)
        acc = gacc = None
        for j in range(NT):
            x = rows_bf16(xa32, j, r0, 128).astype(f32)
            t = x * wr[:, 128 * j: 128 * (j + 1)]
            u = x * gw[:, 128 * j: 128 * (j + 1)]
            acc = t if acc is None else acc + t
            gacc = u if gacc is None else gacc + u
        g = _sigmoid(jnp.sum(gacc, axis=1, keepdims=True))
        gate[r0 // T][pl.ds(r0 % T, 128), :] = jnp.broadcast_to(g, (128, 128))
        r = jnp.sum(acc.T, axis=0, keepdims=True)
        r = r.astype(bf16).astype(f32) + 0.0
        bits = pltpu.bitcast(r, i32)
        bits = jnp.where(bits < 0, bits ^ 0x7FFF0000, bits)
        pos = r0 + lax.broadcasted_iota(i32, (1, 128), 1)
        rkeys[pl.ds(r0 // 128, 1), :] = bits | (0xFFFF - pos)

    state = {}

    def select():
        keys = rkeys[...]
        k0 = jnp.max(keys)
        k1 = jnp.max(jnp.where(keys == k0, jnp.iinfo(jnp.int32).min, keys))
        state["sel"] = (k0, k1)

    def row_tile(key):
        idx = jnp.clip(0xFFFF - (key & 0xFFFF), 0, S - 1)
        return pl.multiple_of((idx >> 4) << 3, 8), idx & 15

    def x_tile(base):
        return jnp.concatenate(
            [_unpacked(xa32[j, pl.ds(base, 8), :]) for j in range(NT)], axis=1).astype(f32)

    def gather():
        row = lax.broadcasted_iota(i32, (16, D), 0)
        x_sel = jnp.zeros((16, D), f32)
        for n, key in enumerate(state["sel"]):
            base, sub = row_tile(key)
            picked = jnp.sum(jnp.where(row == sub, x_tile(base), 0.0), axis=0, keepdims=True)
            x_sel = jnp.where(row == n, picked, x_sel)
        state["x_sel"] = x_sel.astype(bf16)

    def ffn_up(f0, n, which):
        w_t = wide_bf16(wu32 if which else wg32, 0, f0, n)
        y = lax.dot_general(state["x_sel"], w_t, (((1,), (1,)), ((), ())),
                            preferred_element_type=f32)
        if which == 0:
            state["g", f0] = y * _sigmoid(y)
        else:
            state["h", f0] = (state["g", f0] * y).astype(bf16)

    def ffn_down(f0, n):
        w = wide_bf16(wd32, 0, f0, n)
        y = jnp.dot(state["h", f0], w, preferred_element_type=f32)
        state["y"] = y if f0 == 0 else state["y"] + y

    def scatter():
        row = lax.broadcasted_iota(i32, (16, D), 0)
        for n, key in enumerate(state["sel"]):
            base, sub = row_tile(key)
            kv = jnp.full((1, D), key, i32) & -65536
            r = pltpu.bitcast(jnp.where(kv < 0, kv ^ 0x7FFF0000, kv), f32)
            upd = state["y"][n: n + 1] * _sigmoid(r)
            tile = x_tile(base)
            tile = jnp.where(row == sub, tile + upd, tile).astype(bf16)
            for j in range(NT):
                xa32[j, pl.ds(base, 8), :] = _packed(tile[:, 128 * j: 128 * (j + 1)])

    def finish(r0, n, j):
        c, r = divmod(r0, T)
        a = matmul(ob[c], r, n, 3 * NT + j)
        b = rows_bf16(xa32, j, r0, n).astype(f32)
        mixed = b + gate[c][pl.ds(r, n), :] * (a - b)
        block = max(k for k, start_row in enumerate(SENDS) if start_row <= r0)
        last = r0 + n == S and j == NT - 1
        if last:
            tie = jnp.concatenate([state["clock"] & state["zero"]] * (n // 8), axis=0)
            mixed = pltpu.bitcast(pltpu.bitcast(mixed, u32) | tie, f32)
        outb[block][pl.ds(r0 - SENDS[block], n), pl.ds(128 * j, 128)] = mixed.astype(bf16)
        if block > 0 and r0 == SENDS[block] and j == SEND_AT:
            cp_out[block - 1].start()
        if last:
            cp_out[block].start()

    fns = dict(
        project=project, finish=finish,
        permute_wqkv=permute_wqkv, permute_wo=permute_wo, permute_x=permute_x,
        scores=scores, softmax=softmax, mix_values=mix_values, router=router,
        select=lambda: select() or gather(), ffn_up=ffn_up, ffn_down=ffn_down, scatter=scatter)
    arrivals = dict(wq_x0=cp_w[0] + cp_x[0], wk_x1=cp_w[1] + cp_x[1],
                    wv_x2=cp_w[2] + cp_vec + cp_x[2], wo_x3=cp_x[3] + cp_wo,
                    ffn=cp_wg + cp_wu, wd=cp_wd)
    for copies in arrivals.values():
        start(copies)
    zeros[...] = jnp.zeros((8, 128), i32)
    state["zero"] = clock = pltpu.bitcast(jnp.full((8, 128), jnp.max(zeros[...]), i32), u32)
    credit = 0
    for waits, tasks in _schedule():
        for name in waits:
            wait(arrivals[name])
        names = [task[0] for task in tasks]
        ticks = (TICK * (names.count("project") + names.count("finish"))
                 - 2 * names.count("softmax") - RT * names.count("router"))
        ticks = max(ticks, 0) / max(names.count("scores") + names.count("mix_values"), 1)
        for name, *args in tasks:
            res = fns[name](*args)
            if res is not None:
                clock = clock ^ pltpu.bitcast(res[-8:], u32)
                credit += ticks
                while credit >= 1:
                    clock = pltpu.roll(clock, 1, 1)
                    credit -= 1
                state["clock"] = clock
    wait(cp_out)


@jax.jit
def pallas_gated_mix__sliding_local_dilated__moe_arch_mod__prompt_kernel(
    A_x: jax.Array,
    A_wqkv: jax.Array,
    A_wo: jax.Array,
    B_x: jax.Array,
    B_w_r: jax.Array,
    B_w_gate: jax.Array,
    B_w_up: jax.Array,
    B_w_down: jax.Array,
    gate_w: jax.Array,
):
    del B_x
    hbm = pl.BlockSpec(memory_space=pltpu.HBM)
    vmem = pltpu.VMEM
    out = pl.pallas_call(
        _kernel,
        in_specs=[hbm] * 8,
        out_specs=hbm,
        out_shape=jax.ShapeDtypeStruct((S, D), bf16),
        scratch_shapes=[
            vmem((NT, S, 128), bf16),
            vmem((3 * NT, D, 128), bf16),
            vmem((NT, D, 128), bf16),
            vmem((NT, F, 128), bf16),
            vmem((NT, F, 128), bf16),
            vmem((NT, F, 128), bf16),
            vmem((D,), bf16),
            vmem((D,), bf16),
            vmem((S // 128, 128), i32),
            [vmem((D, 128), u32)] * 9,
            [vmem((D, 128), f32)] * NT,
            vmem((4 * NT + 2 * NC * NT, D // 2, 128), u32),
            vmem((NC * (3 * NT + 2 * W), HALO + T, 128), f32),
            [vmem((T, 128), f32)] * NC,
            [vmem((n, D), bf16) for _, n in SEND_ROWS],
            vmem((8, 128), i32),
            pltpu.SemaphoreType.DMA((128,)),
        ],
        compiler_params=pltpu.CompilerParams(vmem_limit_bytes=100 * 1024 * 1024),
    )(A_x.reshape(S, D), A_wqkv, A_wo, B_w_r, B_w_gate.T, B_w_up.T, B_w_down, gate_w)
    return out.reshape(1, S, D)
```
